```python
import jax
import jax.numpy as jnp

def _softmax(x, axis=-1):
    return jax.nn.softmax(x, axis=axis)
def _gelu(x):
    return jax.nn.gelu(x, approximate=True)
def _silu(x):
    return jax.nn.silu(x)
def _sigmoid(x):
    return jax.nn.sigmoid(x)
def _layernorm(x, axis=-1, eps=1e-5):
    m = jnp.mean(x, axis=axis, keepdims=True)
    v = jnp.var(x, axis=axis, keepdims=True)
    return (x - m) / jnp.sqrt(v + eps)
def _scatter_add(tgt, idx, src, axis=0):
    return tgt.at[idx].add(src)
def _segment_sum(src, seg, n):
    return jax.ops.segment_sum(src, seg, n)
class _Rng:
    def __init__(self, key):
        self._k = key
    def _next(self):
        self._k, sub = jax.random.split(self._k)
        return sub
    def normal(self, shape):
        return jax.random.normal(self._next(), shape, dtype=jnp.bfloat16)
    def randint(self, lo, hi, shape):
        return jax.random.randint(self._next(), shape, lo, hi, dtype=jnp.int32)
    def uniform(self, shape, lo=0.0, hi=1.0):
        return jax.random.uniform(self._next(), shape, jnp.bfloat16, lo, hi)
    def permutation(self, n):
        return jax.random.permutation(self._next(), n)


kernel_name = 'interleave_layers__sliding_local_dilated__linear_kernel_hedgehog__prompt'

def setup_inputs():
    _rng = _Rng(jax.random.key(int.from_bytes(__import__("os").urandom(4), "little")))
    _w = (lambda a: (lambda t: t.astype(jnp.bfloat16) if jnp.issubdtype(t.dtype, jnp.floating) else t)(jnp.asarray(a)))
    def _A_setup():
        B, S, D = 1, 2048, 1024
        return {
            "x": _w((lambda *s: _rng.normal(s) * 0.05)(B, S, D)),
            "wqkv": _w((lambda *s: _rng.normal(s) * 0.05)(D, 3 * D)),
            "wo": _w((lambda *s: _rng.normal(s) * 0.05)(D, D)),
        }
    _A_in = _A_setup()

    def _B_setup():
        B, S, D, H = 1, 2048, 1024, 32
        Dh = D // H
        return {
            "x": _w((lambda *s: _rng.normal(s) * 0.05)(B, S, D)),
            "wqkv": _w((lambda *s: _rng.normal(s) * 0.05)(D, 3 * D)),
            "w_phi": _w((lambda *s: _rng.normal(s) * 0.05)(H, Dh, Dh) * (Dh ** -0.5)),
            "wo": _w((lambda *s: _rng.normal(s) * 0.05)(D, D)),
        }
    _B_in = _B_setup()

    return {
        "A_x": _A_in["x"],
        "A_wqkv": _A_in["wqkv"],
        "A_wo": _A_in["wo"],
        "B_x": _B_in["x"],
        "B_wqkv": _B_in["wqkv"],
        "B_w_phi": _B_in["w_phi"],
        "B_wo": _B_in["wo"],
    }

def reference(A_x, A_wqkv, A_wo, B_x, B_wqkv, B_w_phi, B_wo):
    def _A_ref(x, wqkv, wo):
        B, S, D = x.shape
        H = 32; Dh = D // H
        W, dil = 8, 2
        qkv = (lambda x, *d: x.transpose(*d))((x @ wqkv).reshape(B, S, 3, H, Dh), 2, 0, 3, 1, 4)
        q, k, v = qkv[0], qkv[1], qkv[2]
        scale = Dh ** -0.5
        pos = jnp.arange(S)
        off = jnp.arange(W) * dil
        idx = pos[:, None] - off[None, :]
        mask = idx >= 0
        idx_c = jnp.where(mask, idx, 0).reshape(-1)
        kg = k[:, :, idx_c, :].reshape(B, H, S, W, Dh)
        vg = v[:, :, idx_c, :].reshape(B, H, S, W, Dh)
        logits = jnp.einsum("bhsd,bhswd->bhsw", q, kg) * scale
        logits = jnp.where(mask[None, None, :, :], logits, -1e9)
        attn = _softmax(logits, axis=-1)
        o = jnp.einsum("bhsw,bhswd->bhsd", attn, vg)
        return (lambda x, *d: x.transpose(*d))(o, 0, 2, 1, 3).reshape(B, S, D) @ wo

    def _B_ref(x, wqkv, w_phi, wo):
        B, S, D = x.shape
        H = 32; Dh = D // H
        qkv = (lambda x, *d: x.transpose(*d))((x @ wqkv).reshape(B, S, 3, H, Dh), 2, 0, 3, 1, 4)
        q, k, v = qkv[0], qkv[1], qkv[2]
        pq = jnp.einsum("bhsd,hdf->bhsf", q, w_phi)
        pk = jnp.einsum("bhsd,hdf->bhsf", k, w_phi)
        phi_q = jnp.concatenate([_softmax(pq, axis=-1), _softmax(-pq, axis=-1)], axis=-1)
        phi_k = jnp.concatenate([_softmax(pk, axis=-1), _softmax(-pk, axis=-1)], axis=-1)
        kv = jnp.einsum("bhsf,bhsd->bhfd", phi_k, v)
        z  = jnp.einsum("bhsf->bhf", phi_k)
        num = jnp.einsum("bhqf,bhfd->bhqd", phi_q, kv)
        den = jnp.einsum("bhqf,bhf->bhq", phi_q, z)[..., None] + 1e-6
        o = num / den
        return (lambda x, *d: x.transpose(*d))(o, 0, 2, 1, 3).reshape(B, S, D) @ wo

    x = A_x
    x = x + _A_ref(_layernorm(x, axis=-1), A_wqkv, A_wo)
    x = x + _B_ref(_layernorm(x, axis=-1), B_wqkv, B_w_phi, B_wo)
    x = x + _A_ref(_layernorm(x, axis=-1), A_wqkv, A_wo)
    x = x + _B_ref(_layernorm(x, axis=-1), B_wqkv, B_w_phi, B_wo)
    return x
```

```python
import jax
import jax.numpy as jnp
from jax import lax
import jax.experimental.pallas as pl
import jax.experimental.pallas.tpu as pltpu

S, D, H, DH, W, DIL = 2048, 1024, 32, 32, 8, 2
T = 128
R = S // T
G = D // T
NC = 512
F32, BF16 = jnp.float32, jnp.bfloat16
LOG2E = 1.4426950408889634
NT = (((1,), (1,)), ((), ()))


def _dot(a, b):
    return jnp.dot(a, b, preferred_element_type=F32)


def _sub_allreduce(x, op):
    for d in (4, 2, 1):
        x = op(x, pltpu.roll(x, d, 0))
    return x


def _fold4(x, op):
    return op(op(x[0:8], x[8:16]), op(x[16:24], x[24:32]))


def _normalize(x):
    m = jnp.sum(x.reshape(D // 8, 8, T), axis=0)
    m = _sub_allreduce(m, jnp.add) * (1.0 / D)
    c = x.reshape(D // 8, 8, T) - m
    v = _sub_allreduce(jnp.sum(c * c, axis=0), jnp.add) * (1.0 / D)
    return (c * lax.rsqrt(v + 1e-5)).reshape(D, T).astype(BF16)


def _kernel(x_hbm, awqkv_hbm, awo_hbm, bwqkv_hbm, phi_hbm, bwo_hbm, out_hbm,
            xio, stage, phis, xt, xn, ot, wa, wao, wb, wbo, buf0, buf1,
            ph0, ph1, kvt, sems):

    def wcopy(k):
        src = (awqkv_hbm, awqkv_hbm, awqkv_hbm, awo_hbm,
               bwqkv_hbm, bwqkv_hbm, bwqkv_hbm, bwo_hbm)[k]
        if k % 4 != 3:
            src = src.at[:, pl.ds((k % 4) * D, D)]
        return pltpu.make_async_copy(src, stage.at[k], sems.at[k])

    xcopy = [pltpu.make_async_copy(x_hbm.at[:, pl.ds(j * T, T)], xio.at[j],
                                   sems.at[8]) for j in range(G)]
    pcopy = pltpu.make_async_copy(phi_hbm, phis, sems.at[9])
    for cp in xcopy:
        cp.start()
    for k in range(8):
        wcopy(k).start()
    pcopy.start()

    for cp in xcopy:
        cp.wait()
    xio32 = xio.bitcast(jnp.uint32)
    with jax.named_scope("load_x"):
        for m in range(R // 2):
            u = jnp.concatenate([xio32[j, pl.ds(m, T, stride=R // 2), :]
                                 for j in range(G)], axis=1)
            for par in range(2):
                bits = (u << 16) if par == 0 else (u & jnp.uint32(0xFFFF0000))
                t = pltpu.bitcast(bits, F32).T
                cols = slice((2 * m + par) * T, (2 * m + par + 1) * T)
                xt[:, cols] = t
                xn[:, cols] = _normalize(t)

    def wt(k, g):
        return stage[k, :, pl.ds(pl.multiple_of(g * T, T), T)].T

    with jax.named_scope("prep_a"):
        for k in range(4):
            wcopy(k).wait()

        def prep_a(g, _):
            for k in range(3):
                wa[g, k * T:(k + 1) * T, :] = wt(k, g)
            wao[pl.ds(pl.multiple_of(g * T, T), T), :] = wt(3, g)
        lax.fori_loop(0, G, prep_a, None)

    sub = lax.broadcasted_iota(jnp.int32, (8, T), 0)
    lane = lax.broadcasted_iota(jnp.int32, (8, T), 1)
    bufs = (buf0, buf1)
    phb = (ph0, ph1)

    def compact(ps):
        for d in (4, 2, 1):
            clear = (sub & d) == 0
            nxt = []
            for j in range(d):
                a, b = ps[j], ps[j + d]
                if d == 4:
                    nxt.append(jnp.where(clear, a, b)
                               + pltpu.roll(jnp.where(clear, b, a), 4, 0))
                else:
                    nxt.append(jnp.where(clear, a + pltpu.roll(a, 8 - d, 0),
                                         b + pltpu.roll(b, d, 0)))
            ps = nxt
        return ps[0]

    def a_mm(g, buf):
        for c in range(S // NC):
            cols = slice(c * NC, (c + 1) * NC)
            buf[:, cols] = _dot(wa[g], xn[:, cols])
        for t in range(DIL, R):
            buf[T:, (R + t) * T:(R + t + 1) * T] = pltpu.roll(
                buf[T:, t * T:(t + 1) * T], 1, 1)

    def a_attn(g, buf):
        row = pl.multiple_of(g * T, T)
        for h in range(T // DH):
            for r in range(R):
                def win(sec, w):
                    t = (r - DIL * w) % (2 * R)
                    return buf[sec * T + h * DH:sec * T + (h + 1) * DH,
                               t * T:(t + 1) * T]
                q = win(0, 0)
                lg = compact([_fold4(q * win(1, w), jnp.add) for w in range(W)])
                lg = lg * (DH ** -0.5)
                if r < DIL * (W - 1):
                    lg = jnp.where((lane == 0) & (sub * DIL > r), -1e9, lg)
                e = jnp.exp(lg - _sub_allreduce(lg, jnp.maximum))
                p = e / _sub_allreduce(e, jnp.add)
                o = None
                for w in range(W):
                    term = (win(2, w).reshape(DH // 8, 8, T)
                            * jnp.broadcast_to(p[w:w + 1], (8, T)))
                    o = term if o is None else o + term
                ot[pl.ds(row + h * DH, DH), r * T:(r + 1) * T] = (
                    o.reshape(DH, T).astype(BF16))

    def pipeline(mm, ew):
        mm(0, 0)

        def body(i, _):
            mm(2 * i + 1, 1)
            ew(2 * i, 0)
            mm(2 * i + 2, 0)
            ew(2 * i + 1, 1)
        lax.fori_loop(0, G // 2 - 1, body, None)
        mm(G - 1, 1)
        ew(G - 2, 0)
        ew(G - 1, 1)

    def out_proj(wo, last):
        def body(c, _):
            c0 = pl.multiple_of(c * 2 * NC, 2 * NC)
            for j in range(2):
                y = _dot(wo[...], ot[:, pl.ds(c0 + j * NC, NC)])
                for k in range(NC // T):
                    cols = pl.ds(c0 + j * NC + k * T, T)
                    x = xt[:, cols] + y[:, k * T:(k + 1) * T]
                    xt[:, cols] = x
                    xn[:, cols] = _normalize(x)
        lax.fori_loop(0, S // (2 * NC), body, None)

    def layer_a():
        with jax.named_scope("a_attn"):
            pipeline(lambda g, s: a_mm(g, bufs[s]),
                     lambda g, s: a_attn(g, bufs[s]))
        with jax.named_scope("a_out"):
            out_proj(wao, False)

    def feature_map(src, dst):
        for h in range(T // DH):
            for r in range(R):
                cols = slice(r * T, (r + 1) * T)
                p = src[h * DH:(h + 1) * DH, cols]
                for sgn, op in ((0, jnp.maximum), (1, jnp.minimum)):
                    m = _sub_allreduce(_fold4(p, op), op)
                    p3 = p.reshape(DH // 8, 8, T)
                    e = jnp.exp(m - p3 if sgn else p3 - m)
                    inv = 1.0 / _sub_allreduce(jnp.sum(e, axis=0), jnp.add)
                    dst[sgn * T + h * DH:sgn * T + (h + 1) * DH, cols] = (
                        (e * inv).reshape(DH, T).astype(BF16))

    def bk_mm(g, buf):
        for c in range(S // NC):
            cols = slice(c * NC, (c + 1) * NC)
            buf[:2 * T, cols] = _dot(wb[g, T:, :], xn[:, cols])

    rowh = lax.broadcasted_iota(jnp.int32, (T + 16, 2 * T), 0)
    colh = (lax.broadcasted_iota(jnp.int32, (T + 16, 2 * T), 1) % T) // DH
    diag = jnp.where(rowh < T, rowh // DH, rowh - T) == colh

    def bk_ew(g, s):
        buf, ph = bufs[s], phb[s]
        feature_map(buf, ph)
        v = jnp.concatenate([buf[T:2 * T, :S].astype(BF16),
                             jnp.ones((16, S), BF16)], axis=0)
        kv = lax.dot_general(v, ph[...], NT, preferred_element_type=F32)
        kvt[g] = jnp.where(diag, kv, 0.0).astype(BF16)

    def bq_mm(g, buf):
        for c in range(S // NC):
            cols = slice(c * NC, (c + 1) * NC)
            buf[:T, cols] = _dot(wb[g, :T, :], xn[:, cols])

    def bq_ew(g, s):
        buf, ph = bufs[s], phb[s]
        row = pl.multiple_of(g * T, T)
        feature_map(buf, ph)
        for c in range(S // NC):
            cols = slice(c * NC, (c + 1) * NC)
            nd = _dot(kvt[g], ph[:, cols])
            inv = 1.0 / (nd[T:T + 8] + 1e-6)
            for h in range(T // DH):
                ot[pl.ds(row + h * DH, DH), cols] = (
                    nd[h * DH:(h + 1) * DH] * inv[h:h + 1]).astype(BF16)

    def layer_b():
        with jax.named_scope("b_kv"):
            pipeline(lambda g, s: bk_mm(g, bufs[s]), bk_ew)
        with jax.named_scope("b_q"):
            pipeline(lambda g, s: bq_mm(g, bufs[s]), bq_ew)
        with jax.named_scope("b_out"):
            out_proj(wbo, False)

    layer_a()

    with jax.named_scope("prep_b"):
        for k in range(4, 8):
            wcopy(k).wait()
        pcopy.wait()

        def prep_b(g, _):
            rows = phis[pl.ds(pl.multiple_of(g * T, T), T), :]
            bd = jnp.where(diag[:T, :T], jnp.concatenate([rows] * 4, axis=1), 0)
            bdt = bd.astype(F32).T.astype(BF16)
            for k in range(2):
                wb[g, k * T:(k + 1) * T, :] = _dot(bdt, wt(4 + k, g)).astype(BF16)
            wb[g, 2 * T:, :] = wt(6, g)
            wbo[pl.ds(pl.multiple_of(g * T, T), T), :] = wt(7, g)
        lax.fori_loop(0, G, prep_b, None)

    layer_b()
    layer_a()
    layer_b()

    with jax.named_scope("store"):
        for j in range(G):
          for m in range(R // 2):
            def bits(r):
                t = xt[j * T:(j + 1) * T, r * T:(r + 1) * T]
                t = t.astype(BF16).astype(F32).T
                return pltpu.bitcast(t, jnp.uint32)
            xio32[j, pl.ds(m, T, stride=R // 2), :] = (
                (bits(2 * m) >> 16) | bits(2 * m + 1))
        ocopy = [pltpu.make_async_copy(xio.at[j], out_hbm.at[:, pl.ds(j * T, T)],
                                       sems.at[8]) for j in range(G)]
        for cp in ocopy:
            cp.start()
        for cp in ocopy:
            cp.wait()


@jax.jit
def pallas_interleave_layers__sliding_local_dilated__linear_kernel_hedgehog__prompt_kernel(
    A_x, A_wqkv, A_wo, B_x, B_wqkv, B_w_phi, B_wo):
    del B_x
    vmem = pltpu.VMEM
    out = pl.pallas_call(
        _kernel,
        out_shape=jax.ShapeDtypeStruct((S, D), BF16),
        in_specs=[pl.BlockSpec(memory_space=pl.ANY)] * 6,
        out_specs=pl.BlockSpec(memory_space=pl.ANY),
        scratch_shapes=[
            vmem((G, S, T), BF16),
            vmem((8, D, D), BF16),
            vmem((D, DH), BF16),
            vmem((D, S), F32),
            vmem((D, S), BF16),
            vmem((D, S), BF16),
            vmem((G, 3 * T, D), BF16),
            vmem((D, D), BF16),
            vmem((G, 3 * T, D), BF16),
            vmem((D, D), BF16),
            vmem((3 * T, 2 * S), F32),
            vmem((3 * T, 2 * S), F32),
            vmem((2 * T, S), BF16),
            vmem((2 * T, S), BF16),
            vmem((G, T + 16, 2 * T), BF16),
            pltpu.SemaphoreType.DMA((10,)),
        ],
        compiler_params=pltpu.CompilerParams(vmem_limit_bytes=100 * 1024 * 1024),
    )(A_x.reshape(S, D), A_wqkv, A_wo, B_wqkv, B_w_phi.reshape(D, DH), B_wo)
    return out.reshape(1, S, D)
```

```python
import functools

import jax
import jax.numpy as jnp
from jax import lax
import jax.experimental.pallas as pl
import jax.experimental.pallas.tpu as pltpu

S, D, H, DH, W, DIL = 2048, 1024, 32, 32, 8, 2
T = 128
R = S // T
G = D // T
NC = 512
F32, BF16 = jnp.float32, jnp.bfloat16
LOG2E = 1.4426950408889634
NT = (((1,), (1,)), ((), ()))


def _dot(a, b):
    return jnp.dot(a, b, preferred_element_type=F32)


def _rows(row, n):
    if isinstance(row, int):
        return pl.ds(row // 2, n // 2)
    return pl.ds(pl.multiple_of(row // 2, 8), n // 2)


def _ld(ref, g, row, n, cols=slice(None)):
    idx = (_rows(row, n), cols) if g is None else (g, _rows(row, n), cols)
    return pltpu.bitcast(ref[idx], BF16)


def _st(ref, g, row, cols, val):
    rows = _rows(row, val.shape[0])
    idx = (rows, cols) if g is None else (g, rows, cols)
    ref[idx] = pltpu.bitcast(val.astype(BF16), jnp.uint32)


def _mix(*lists):
    items = [((i + 0.5) / len(l), j, f)
             for j, l in enumerate(lists) for i, f in enumerate(l)]
    for _, _, f in sorted(items, key=lambda t: t[:2]):
        f()


def _sub_allreduce(x, op):
    for d in (4, 2, 1):
        x = op(x, pltpu.roll(x, d, 0))
    return x


def _fold4(x, op):
    return op(op(x[0:8], x[8:16]), op(x[16:24], x[24:32]))


def _normalize(x):
    m = jnp.sum(x.reshape(D // 8, 8, T), axis=0)
    m = _sub_allreduce(m, jnp.add) * (1.0 / D)
    c = x.reshape(D // 8, 8, T) - m
    v = _sub_allreduce(jnp.sum(c * c, axis=0), jnp.add) * (1.0 / D)
    return (c * lax.rsqrt(v + 1e-5)).reshape(D, T).astype(BF16)


def _kernel(x_hbm, awqkv_hbm, awo_hbm, bwqkv_hbm, phi_hbm, bwo_hbm, out_hbm,
            xio, stage, phis, xt, xn, ot, wa, wao, wb, wbo, buf0, buf1,
            ph0, ph1, kvt, kvacc, sems):

    def wcopy(k, lo, n, sem):
        src = (awqkv_hbm, awqkv_hbm, awqkv_hbm, awo_hbm,
               bwqkv_hbm, bwqkv_hbm, bwqkv_hbm, bwo_hbm)[k]
        src = src.at[:, pl.ds((k % 4) * D * (k % 4 != 3) + lo, n)]
        return pltpu.make_async_copy(src, stage.at[k, :, pl.ds(lo, n)],
                                     sems.at[sem])

    xcopy = [pltpu.make_async_copy(x_hbm.at[:, pl.ds(j * T, T)], xio.at[j],
                                   sems.at[0]) for j in range(G)]
    first = [wcopy(k, 0, T, 1) for k in range(3)]
    second = [wcopy(k, T, T, 2) for k in range(3)]
    rest_a = [wcopy(k, 2 * T, D - 2 * T, 3) for k in range(3)]
    rest_a.append(wcopy(3, 0, D, 3))
    all_b = [wcopy(k, 0, D, 4) for k in range(4, 8)]
    all_b.append(pltpu.make_async_copy(phi_hbm, phis, sems.at[4]))

    def start(cps):
        for cp in cps:
            cp.start()

    def wait(cps):
        for cp in cps:
            cp.wait()

    xio32 = xio.bitcast(jnp.uint32)
    hi_mask = jnp.uint32(0xFFFF0000)

    def load_x(r):
        u = jnp.concatenate([xio32[j, pl.ds(r // 2, T, stride=R // 2), :]
                             for j in range(G)], axis=1)
        t = pltpu.bitcast((u & hi_mask) if r % 2 else (u << 16), F32).T
        cols = slice(r * T, (r + 1) * T)
        xt[:, cols] = t
        _st(xn, None, 0, cols, _normalize(t))

    def wt(k, g):
        c0 = g * T if isinstance(g, int) else pl.multiple_of(g * T, T)
        return stage[k, :, pl.ds(c0, T)].T

    def prep(k, g):
        dst, gi, row = (((wa, g, k * T),) * 3 + ((wao, None, g * T),)
                        + ((wb, g, k * T - 4 * T),) * 3 + ((wbo, None, g * T),))[k]
        w = wt(k, g)
        if k in (4, 5):
            r0 = g * T if isinstance(g, int) else pl.multiple_of(g * T, T)
            rows = phis[pl.ds(r0, T), :]
            bd = jnp.where(diag[:T, :T], jnp.concatenate([rows] * 4, axis=1), 0)
            w = _dot(bd.astype(F32).T.astype(BF16), w)
        _st(dst, gi, row, slice(None), w)

    def preps(*kg):
        return [functools.partial(prep, k, g) for k, g in kg]

    sub = lax.broadcasted_iota(jnp.int32, (8, T), 0)
    lane = lax.broadcasted_iota(jnp.int32, (8, T), 1)
    bufs = (buf0, buf1)
    phb = (ph0, ph1)

    def compact(ps):
        for d in (4, 2, 1):
            clear = (sub & d) == 0
            nxt = []
            for j in range(d):
                a, b = ps[j], ps[j + d]
                if d == 4:
                    nxt.append(jnp.where(clear, a, b)
                               + pltpu.roll(jnp.where(clear, b, a), 4, 0))
                else:
                    nxt.append(jnp.where(clear, a + pltpu.roll(a, 8 - d, 0),
                                         b + pltpu.roll(b, d, 0)))
            ps = nxt
        return ps[0]

    def proj(w, g, row0, nblk, buf):
        def unit(k, c):
            cols = slice(c * NC, (c + 1) * NC)
            wk = _ld(w, g, row0 + k * T, T)
            buf[k * T:(k + 1) * T, cols] = _dot(wk, _ld(xn, None, 0, D, cols))
        return [functools.partial(unit, k, c)
                for c in range(S // NC) for k in range(nblk)]

    def a_attn(g, buf, tail=False):
        def shift(h):
            for sec in (1, 2):
                rows = slice(sec * T + h * DH, sec * T + (h + 1) * DH)
                for t in range(DIL, R):
                    buf[rows, (R + t) * T:(R + t + 1) * T] = pltpu.roll(
                        buf[rows, t * T:(t + 1) * T], 1, 1)

        def unit(h, r):
            def win(sec, w):
                t = (r - DIL * w) % (2 * R)
                return buf[sec * T + h * DH:sec * T + (h + 1) * DH,
                           t * T:(t + 1) * T]
            q = win(0, 0)
            lg = compact([_fold4(q * win(1, w), jnp.add) for w in range(W)])
            lg = lg * (DH ** -0.5)
            if r < DIL * (W - 1):
                lg = jnp.where((lane == 0) & (sub * DIL > r), -1e9, lg)
            e = jnp.exp(lg - _sub_allreduce(lg, jnp.maximum))
            p = e / _sub_allreduce(e, jnp.add)
            o = None
            for w in range(W):
                term = (win(2, w).reshape(DH // 8, 8, T)
                        * jnp.broadcast_to(p[w:w + 1], (8, T)))
                o = term if o is None else o + term
            _st(ot, None, g * T + h * DH, slice(r * T, (r + 1) * T),
                o.reshape(DH, T))
        out = []
        if tail:
            return ([functools.partial(shift, h) for h in range(T // DH)]
                    + [functools.partial(unit, h, r)
                       for r in range(R) for h in range(T // DH)])
        for h in range(T // DH):
            out.append(functools.partial(shift, h))
            out += [functools.partial(unit, h, r) for r in reversed(range(R))]
        return out

    def pipeline(mm, ew, extra=lambda g: []):
        def body(i, _):
            _mix(mm(2 * i + 1, 1), ew(2 * i, 0), extra(2 * i + 1))
            _mix(mm(2 * i + 2, 0), ew(2 * i + 1, 1), extra(2 * i + 2))
        lax.fori_loop(0, G // 2 - 1, body, None)
        _mix(mm(G - 1, 1), ew(G - 2, 0), extra(G - 1))

    def wo_unit(wo, k, c):
        cols = slice(c * NC, (c + 1) * NC)
        y = _dot(_ld(wo, None, k * T, T), _ld(ot, None, 0, D, cols))
        xt[_rows(2 * k * T, 2 * T), cols] += y

    def ln(c):
        def unit(r):
            cols = slice(r * T, (r + 1) * T)
            _st(xn, None, 0, cols, _normalize(xt[:, cols]))
        n = NC // T
        return [functools.partial(unit, r) for r in range(c * n, c * n + n)]

    def out_proj(wo, tail, nxt, extra=()):
        mm = lambda c: [functools.partial(wo_unit, wo, k, c) for k in range(G)]
        n = len(tail) * 3 // 8
        _mix(tail[:n + 1])
        _mix(mm(0), tail[n + 1:])
        for c in range(1, S // NC):
            _mix(mm(c), ln(c - 1), extra)
            extra = ()
        _mix(nxt[:len(nxt) // 2], ln(S // NC - 1))
        _mix(nxt[len(nxt) // 2:])

    a_mm = lambda g, s: proj(wa, g, 0, 3, bufs[s])
    a_ew = lambda g, s: a_attn(g, bufs[s])
    bk_mm = lambda g, s: proj(wb, g, T, 2, bufs[s])
    bq_mm = lambda g, s: proj(wb, g, 0, 1, bufs[s])

    def feature_map(src, dst, c):
        def unit(h, r):
            cols = slice(r * T, (r + 1) * T)
            p = src[h * DH:(h + 1) * DH, cols]
            for sgn, op in ((0, jnp.maximum), (1, jnp.minimum)):
                m = _sub_allreduce(_fold4(p, op), op)
                p3 = p.reshape(DH // 8, 8, T)
                e = jnp.exp(m - p3 if sgn else p3 - m)
                inv = 1.0 / _sub_allreduce(jnp.sum(e, axis=0), jnp.add)
                _st(dst, None, sgn * T + h * DH, cols, (e * inv).reshape(DH, T))
        n = NC // T
        return [functools.partial(unit, h, r)
                for r in range(c * n, c * n + n) for h in range(T // DH)]

    rowh = lax.broadcasted_iota(jnp.int32, (T + 16, 2 * T), 0)
    colh = (lax.broadcasted_iota(jnp.int32, (T + 16, 2 * T), 1) % T) // DH
    diag = jnp.where(rowh < T, rowh // DH, rowh - T) == colh

    def skew(fm, mm):
        out = []
        for c in range(S // NC):
            f = fm(c)
            out += f[:len(f) // 2]
            if c:
                out.append(functools.partial(mm, c - 1))
            out += f[len(f) // 2:]
        return out + [functools.partial(mm, S // NC - 1)]

    def bk_ew(g, s):
        buf, ph = bufs[s], phb[s]

        def mm(c):
            cols = slice(c * NC, (c + 1) * NC)
            v = jnp.concatenate([buf[T:2 * T, cols].astype(BF16),
                                 jnp.ones((16, NC), BF16)], axis=0)
            kv = lax.dot_general(v, _ld(ph, None, 0, 2 * T, cols), NT,
                                 preferred_element_type=F32)
            if c:
                kv = kv + kvacc[...]
            if c < S // NC - 1:
                kvacc[...] = kv
            else:
                _st(kvt, g, 0, slice(None), jnp.where(diag, kv, 0.0))
        return skew(functools.partial(feature_map, buf, ph), mm)

    def bq_ew(g, s):
        buf, ph = bufs[s], phb[s]

        def mm(c):
            cols = slice(c * NC, (c + 1) * NC)
            nd = _dot(_ld(kvt, g, 0, T + 16), _ld(ph, None, 0, 2 * T, cols))
            inv = 1.0 / (nd[T:T + 8] + 1e-6)
            for h in range(T // DH):
                _st(ot, None, g * T + h * DH, cols,
                    nd[h * DH:(h + 1) * DH] * inv[h:h + 1])
        return skew(functools.partial(feature_map, buf, ph), mm)

    def store(j):
        def unit(m):
            def bits(r):
                t = xt[_rows(2 * j * T, 2 * T), r * T:(r + 1) * T]
                return pltpu.bitcast(t.astype(BF16).astype(F32).T, jnp.uint32)
            xio32[j, pl.ds(m, T, stride=R // 2), :] = (
                (bits(2 * m) >> 16) | bits(2 * m + 1))
        return [functools.partial(unit, m) for m in range(R // 2)]

    def ocopy(j):
        c0 = j * T if isinstance(j, int) else pl.multiple_of(j * T, T)
        return pltpu.make_async_copy(xio.at[j], out_hbm.at[:, pl.ds(c0, T)],
                                     sems.at[5])

    def final_proj(tail):
        mm = lambda k: [functools.partial(wo_unit, wbo, k, c)
                        for c in range(S // NC)]
        _mix(tail)
        _mix(mm(0))
        _mix(mm(1), store(0))

        def body(k, _):
            ocopy(k - 2).start()
            _mix(mm(k), store(k - 1))
        lax.fori_loop(2, G, body, None)
        ocopy(G - 2).start()
        _mix(store(G - 1))
        pl.when(pl.program_id(0) == 0)(ocopy(G - 1).start)
        wait([ocopy(k) for k in range(G)])

    def layer_b(last):
        with jax.named_scope("b_kv"):
            pipeline(bk_mm, bk_ew, (lambda g: []) if last else
                     (lambda g: preps((5, g), (6, g), (4, g - 1))))
            _mix(bq_mm(0, 0), bk_ew(G - 1, 1), [] if last else preps((4, G - 1)))
        with jax.named_scope("b_q"):
            pipeline(bq_mm, bq_ew, (lambda g: []) if last else
                     (lambda g: preps((7, g - 1))))
        with jax.named_scope("b_out"):
            if last:
                final_proj(bq_ew(G - 1, 1))
            else:
                out_proj(wbo, bq_ew(G - 1, 1), a_mm(0, 0), preps((7, G - 1)))

    with jax.named_scope("wait_x"):
        start(xcopy + first)
        wait(xcopy + first)
        start(second + rest_a)
    with jax.named_scope("load_x"):
        _mix([functools.partial(load_x, r) for r in range(4)],
             preps((0, 0), (1, 0), (2, 0)))
        wait(second)
        _mix(a_mm(0, 0), [functools.partial(load_x, r) for r in range(4, R)]
             , preps((0, 1), (1, 1), (2, 1)))
        wait(rest_a)
        start(all_b)

    def a_prep(g):
        return preps(*([(k, g + 1) for k in range(3)] if not isinstance(g, int) else []),
                     (3, g - 1))

    for last in (False, True):
        with jax.named_scope("a_attn"):
            pipeline(a_mm, a_ew, (lambda g: []) if last else a_prep)
        with jax.named_scope("a_out"):
            if not last:
                wait(all_b)
            out_proj(wao, a_attn(G - 1, bufs[1], True), bk_mm(0, 0),
                     () if last else preps((3, G - 1), (5, 0), (6, 0)))
        layer_b(last)


@jax.jit
def pallas_interleave_layers__sliding_local_dilated__linear_kernel_hedgehog__prompt_kernel(
    A_x, A_wqkv, A_wo, B_x, B_wqkv, B_w_phi, B_wo):
    del B_x
    vmem = pltpu.VMEM
    out = pl.pallas_call(
        _kernel,
        grid=(1,),
        out_shape=jax.ShapeDtypeStruct((S, D), BF16),
        in_specs=[pl.BlockSpec(memory_space=pl.ANY)] * 6,
        out_specs=pl.BlockSpec(memory_space=pl.ANY),
        scratch_shapes=[
            vmem((G, S, T), BF16),
            vmem((8, D, D), BF16),
            vmem((D, DH), BF16),
            vmem((D, S), F32),
            vmem((D // 2, S), jnp.uint32),
            vmem((D // 2, S), jnp.uint32),
            vmem((G, 3 * T // 2, D), jnp.uint32),
            vmem((D // 2, D), jnp.uint32),
            vmem((G, 3 * T // 2, D), jnp.uint32),
            vmem((D // 2, D), jnp.uint32),
            vmem((3 * T, 2 * S), F32),
            vmem((3 * T, 2 * S), F32),
            vmem((T, S), jnp.uint32),
            vmem((T, S), jnp.uint32),
            vmem((G, T // 2 + 8, 2 * T), jnp.uint32),
            vmem((T + 16, 2 * T), F32),
            pltpu.SemaphoreType.DMA((6,)),
        ],
        compiler_params=pltpu.CompilerParams(vmem_limit_bytes=100 * 1024 * 1024),
    )(A_x.reshape(S, D), A_wqkv, A_wo, B_wqkv, B_w_phi.reshape(D, DH), B_wo)
    return out.reshape(1, S, D)
```

```python
import functools

import jax
import jax.numpy as jnp
from jax import lax
import jax.experimental.pallas as pl
import jax.experimental.pallas.tpu as pltpu

S, D, H, DH, W, DIL = 2048, 1024, 32, 32, 8, 2
T = 128
R = S // T
G = D // T
NC = 512
F32, BF16 = jnp.float32, jnp.bfloat16
LOG2E = 1.4426950408889634
NT = (((1,), (1,)), ((), ()))


def _dot(a, b):
    return jnp.dot(a, b, preferred_element_type=F32)


def _rows(row, n):
    if isinstance(row, int):
        return pl.ds(row // 2, n // 2)
    return pl.ds(pl.multiple_of(row // 2, 8), n // 2)


def _ld(ref, g, row, n, cols=slice(None)):
    idx = (_rows(row, n), cols) if g is None else (g, _rows(row, n), cols)
    return pltpu.bitcast(ref[idx], BF16)


def _st(ref, g, row, cols, val):
    rows = _rows(row, val.shape[0])
    idx = (rows, cols) if g is None else (g, rows, cols)
    ref[idx] = pltpu.bitcast(val.astype(BF16), jnp.uint32)


def _mix(*lists):
    items = [((i + 0.5) / len(l), j, f)
             for j, l in enumerate(lists) for i, f in enumerate(l)]
    for _, _, f in sorted(items, key=lambda t: t[:2]):
        f()


def _sub_allreduce(x, op):
    for d in (4, 2, 1):
        x = op(x, pltpu.roll(x, d, 0))
    return x


def _recip(s):
    r = pl.reciprocal(s, approx=True)
    return r * (2.0 - s * r)


def _fold4(x, op):
    return op(op(x[0:8], x[8:16]), op(x[16:24], x[24:32]))


def _normalize(x):
    m = jnp.sum(x.reshape(D // 8, 8, T), axis=0)
    m = _sub_allreduce(m, jnp.add) * (1.0 / D)
    c = x.reshape(D // 8, 8, T) - m
    v = _sub_allreduce(jnp.sum(c * c, axis=0), jnp.add) * (1.0 / D)
    return (c * lax.rsqrt(v + 1e-5)).reshape(D, T).astype(BF16)


def _kernel(x_hbm, awqkv_hbm, awo_hbm, bwqkv_hbm, phi_hbm, bwo_hbm, out_hbm,
            xio, stage, phis, xt, xn, ot, wa, wao, wb, wbo, buf0, buf1,
            ph0, ph1, kvt, kvacc, y0, y1, yf0, yf1, sems):

    def wcopy(k, lo, n, sem):
        src = (awqkv_hbm, awqkv_hbm, awqkv_hbm, awo_hbm,
               bwqkv_hbm, bwqkv_hbm, bwqkv_hbm, bwo_hbm)[k]
        src = src.at[:, pl.ds((k % 4) * D * (k % 4 != 3) + lo, n)]
        return pltpu.make_async_copy(src, stage.at[k, :, pl.ds(lo, n)],
                                     sems.at[sem])

    xcopy = [pltpu.make_async_copy(x_hbm.at[:, pl.ds(j * T, T)], xio.at[j],
                                   sems.at[0]) for j in range(G)]
    first = [wcopy(k, 0, T, 1) for k in range(3)]
    second = [wcopy(k, T, T, 2) for k in range(3)]
    rest_a = [wcopy(k, 2 * T, D - 2 * T, 3) for k in range(3)]
    rest_a.append(wcopy(3, 0, D, 3))
    all_b = [wcopy(k, 0, D, 4) for k in range(4, 8)]
    all_b.append(pltpu.make_async_copy(phi_hbm, phis, sems.at[4]))

    def start(cps):
        for cp in cps:
            cp.start()

    def wait(cps):
        for cp in cps:
            cp.wait()

    xio32 = xio.bitcast(jnp.uint32)
    hi_mask = jnp.uint32(0xFFFF0000)

    def load_x(r):
        u = jnp.concatenate([xio32[j, pl.ds(r // 2, T, stride=R // 2), :]
                             for j in range(G)], axis=1)
        t = pltpu.bitcast((u & hi_mask) if r % 2 else (u << 16), F32).T
        cols = slice(r * T, (r + 1) * T)
        xt[:, cols] = t
        _st(xn, None, 0, cols, _normalize(t))

    def wt(k, g):
        c0 = g * T if isinstance(g, int) else pl.multiple_of(g * T, T)
        return stage[k, :, pl.ds(c0, T)].T

    def prep(k, g):
        dst, gi, row = (((wa, g, k * T),) * 3 + ((wao, None, g * T),)
                        + ((wb, g, k * T - 4 * T),) * 3 + ((wbo, None, g * T),))[k]
        w = wt(k, g)
        if k in (4, 5):
            r0 = g * T if isinstance(g, int) else pl.multiple_of(g * T, T)
            rows = phis[pl.ds(r0, T), :]
            bd = jnp.where(diag[:T, :T], jnp.concatenate([rows] * 4, axis=1), 0)
            w = _dot(bd.astype(F32).T.astype(BF16), w)
        _st(dst, gi, row, slice(None), w)

    def preps(*kg):
        return [functools.partial(prep, k, g) for k, g in kg]

    sub = lax.broadcasted_iota(jnp.int32, (8, T), 0)
    lane = lax.broadcasted_iota(jnp.int32, (8, T), 1)
    bufs = (buf0, buf1)
    ys, yf = (y0, y1), (yf0, yf1)
    phb = (ph0, ph1)

    def compact(ps):
        for d in (4, 2, 1):
            clear = (sub & d) == 0
            nxt = []
            for j in range(d):
                a, b = ps[j], ps[j + d]
                if d == 4:
                    nxt.append(jnp.where(clear, a, b)
                               + pltpu.roll(jnp.where(clear, b, a), 4, 0))
                else:
                    nxt.append(jnp.where(clear, a + pltpu.roll(a, 8 - d, 0),
                                         b + pltpu.roll(b, d, 0)))
            ps = nxt
        return ps[0]

    def proj(w, g, row0, nblk, buf):
        def unit(k, c):
            cols = slice(c * NC, (c + 1) * NC)
            wk = _ld(w, g, row0 + k * T, T)
            buf[k * T:(k + 1) * T, cols] = _dot(wk, _ld(xn, None, 0, D, cols))
        return [functools.partial(unit, k, c)
                for c in range(S // NC) for k in range(nblk)]

    def a_attn(g, buf, tail=False):
        def shift(h):
            for sec in (1, 2):
                rows = slice(sec * T + h * DH, sec * T + (h + 1) * DH)
                for t in range(DIL, R):
                    buf[rows, (R + t) * T:(R + t + 1) * T] = pltpu.roll(
                        buf[rows, t * T:(t + 1) * T], 1, 1)

        def unit(h, r):
            def win(sec, w):
                t = (r - DIL * w) % (2 * R)
                return buf[sec * T + h * DH:sec * T + (h + 1) * DH,
                           t * T:(t + 1) * T]
            q = win(0, 0)
            lg = compact([_fold4(q * win(1, w), jnp.add) for w in range(W)])
            lg = lg * (DH ** -0.5)
            if r < DIL * (W - 1):
                lg = jnp.where((lane == 0) & (sub * DIL > r), -1e9, lg)
            e = jnp.exp(lg - _sub_allreduce(lg, jnp.maximum))
            p = e * _recip(_sub_allreduce(e, jnp.add))
            o = None
            for w in range(W):
                term = (win(2, w).reshape(DH // 8, 8, T)
                        * jnp.broadcast_to(p[w:w + 1], (8, T)))
                o = term if o is None else o + term
            _st(ot, None, g * T + h * DH, slice(r * T, (r + 1) * T),
                o.reshape(DH, T))
        out = []
        if tail:
            return ([functools.partial(shift, h) for h in range(T // DH)]
                    + [functools.partial(unit, h, r)
                       for r in range(R) for h in range(T // DH)])
        for h in range(T // DH):
            out.append(functools.partial(shift, h))
            out += [functools.partial(unit, h, r) for r in reversed(range(R))]
        return out

    def pipeline(mm, ew, extra=lambda g: []):
        def body(i, _):
            _mix(mm(2 * i + 1, 1), ew(2 * i, 0), extra(2 * i + 1))
            _mix(mm(2 * i + 2, 0), ew(2 * i + 1, 1), extra(2 * i + 2))
        lax.fori_loop(0, G // 2 - 1, body, None)
        _mix(mm(G - 1, 1), ew(G - 2, 0), extra(G - 1))

    def wo_unit(wo, k, c, put):
        cols = slice(c * NC, (c + 1) * NC)
        y = _dot(_ld(wo, None, k * T, T), _ld(ot, None, 0, D, cols))
        put(k, c, y)

    def ln(c):
        def tile(r):
            cols = slice(r * T, (r + 1) * T)
            st = {}
            blk = lambda k: xt[k * T:(k + 1) * T, cols].reshape(T // 8, 8, T)

            def mean(k):
                x = (xt[k * T:(k + 1) * T, cols]
                     + ys[c % 2][k * T:(k + 1) * T, (r % n) * T:(r % n + 1) * T])
                xt[k * T:(k + 1) * T, cols] = x
                m = jnp.sum(x.reshape(T // 8, 8, T), axis=0)
                st["m"] = m + st["m"] if k else m
                if k == G - 1:
                    st["m"] = _sub_allreduce(st["m"], jnp.add) * (1.0 / D)

            def var(k):
                d = blk(k) - st["m"]
                v = jnp.sum(d * d, axis=0)
                st["v"] = v + st["v"] if k else v
                if k == G - 1:
                    v = _sub_allreduce(st["v"], jnp.add) * (1.0 / D)
                    st["v"] = lax.rsqrt(v + 1e-5)

            def norm(k):
                y = (blk(k) - st["m"]) * st["v"]
                _st(xn, None, k * T, cols, y.reshape(T, T))
            return [functools.partial(f, k)
                    for f in (mean, var, norm) for k in range(G)]
        n = NC // T
        return [f for r in range(c * n, c * n + n) for f in tile(r)]

    def out_proj(wo, tail, nxt, extra=()):
        def put(k, c, y):
            ys[c % 2][k * T:(k + 1) * T, :] = y
        mm = lambda c: [functools.partial(wo_unit, wo, k, c, put)
                        for k in range(G)]
        n = len(tail) * 3 // 8
        _mix(tail[:n + 1])
        _mix(mm(0), tail[n + 1:])
        for c in range(1, S // NC):
            _mix(mm(c), ln(c - 1), extra[c - 1::3])
        _mix(nxt[:len(nxt) // 2], ln(S // NC - 1))
        _mix(nxt[len(nxt) // 2:])

    a_mm = lambda g, s: proj(wa, g, 0, 3, bufs[s])
    a_ew = lambda g, s: a_attn(g, bufs[s])
    bk_mm = lambda g, s: proj(wb, g, T, 2, bufs[s])
    bq_mm = lambda g, s: proj(wb, g, 0, 1, bufs[s])

    def feature_map(src, dst, c):
        def unit(h, r):
            cols = slice(r * T, (r + 1) * T)
            p = src[h * DH:(h + 1) * DH, cols] * LOG2E
            for sgn, op in ((0, jnp.maximum), (1, jnp.minimum)):
                m = _sub_allreduce(_fold4(p, op), op)
                p3 = p.reshape(DH // 8, 8, T)
                e = jnp.exp2(m - p3 if sgn else p3 - m)
                inv = _recip(_sub_allreduce(jnp.sum(e, axis=0), jnp.add))
                _st(dst, None, sgn * T + h * DH, cols, (e * inv).reshape(DH, T))
        n = NC // T
        return [functools.partial(unit, h, r)
                for r in range(c * n, c * n + n) for h in range(T // DH)]

    rowh = lax.broadcasted_iota(jnp.int32, (T + 16, 2 * T), 0)
    colh = (lax.broadcasted_iota(jnp.int32, (T + 16, 2 * T), 1) % T) // DH
    diag = jnp.where(rowh < T, rowh // DH, rowh - T) == colh

    def skew(fm, mm):
        out = []
        for c in range(S // NC):
            f = fm(c)
            out += f[:2]
            if c:
                out.append(functools.partial(mm, c - 1))
            out += f[2:]
        return out + [functools.partial(mm, S // NC - 1)]

    def bk_ew(g, s):
        buf, ph = bufs[s], phb[s]

        def mm(c):
            cols = slice(c * NC, (c + 1) * NC)
            v = jnp.concatenate([buf[T:2 * T, cols].astype(BF16),
                                 jnp.ones((16, NC), BF16)], axis=0)
            kv = lax.dot_general(v, _ld(ph, None, 0, 2 * T, cols), NT,
                                 preferred_element_type=F32)
            if c:
                kv = kv + kvacc[...]
            if c < S // NC - 1:
                kvacc[...] = kv
            else:
                _st(kvt, g, 0, slice(None), jnp.where(diag, kv, 0.0))
        return skew(functools.partial(feature_map, buf, ph), mm)

    def bq_ew(g, s):
        buf, ph = bufs[s], phb[s]

        def mm(c):
            cols = slice(c * NC, (c + 1) * NC)
            nd = _dot(_ld(kvt, g, 0, T + 16), _ld(ph, None, 0, 2 * T, cols))
            inv = 1.0 / (nd[T:T + 8] + 1e-6)
            for h in range(T // DH):
                _st(ot, None, g * T + h * DH, cols,
                    nd[h * DH:(h + 1) * DH] * inv[h:h + 1])
        return skew(functools.partial(feature_map, buf, ph), mm)

    def store(j, src):
        def unit(m):
            def bits(r):
                t = xt[_rows(2 * j * T, 2 * T), r * T:(r + 1) * T]
                t = t + src[:, r * T:(r + 1) * T]
                return pltpu.bitcast(t.astype(BF16).astype(F32).T, jnp.uint32)
            xio32[j, pl.ds(m, T, stride=R // 2), :] = (
                (bits(2 * m) >> 16) | bits(2 * m + 1))
        return [functools.partial(unit, m) for m in range(R // 2)]

    def ocopy(j):
        c0 = j * T if isinstance(j, int) else pl.multiple_of(j * T, T)
        return pltpu.make_async_copy(xio.at[j], out_hbm.at[:, pl.ds(c0, T)],
                                     sems.at[5])

    def final_proj(tail):
        def mm(k, s):
            def put(k, c, y):
                yf[s][:, c * NC:(c + 1) * NC] = y
            return [functools.partial(wo_unit, wbo, k, c, put)
                    for c in range(S // NC)]
        _mix(tail)
        _mix(mm(0, 0))
        _mix(mm(1, 1), store(0, yf[0]))

        def body(i, _):
            ocopy(2 * i - 2).start()
            _mix(mm(2 * i, 0), store(2 * i - 1, yf[1]))
            _mix(mm(2 * i + 1, 1), store(2 * i, yf[0]))

            @pl.when(pl.program_id(0) == 0)
            def _():
                ocopy(2 * i - 1).start()
        lax.fori_loop(1, G // 2, body, None)
        ocopy(G - 2).start()
        _mix(store(G - 1, yf[1]))
        pl.when(pl.program_id(0) == 0)(ocopy(G - 1).start)
        wait([ocopy(k) for k in range(G)])

    def layer_b(last):
        with jax.named_scope("b_kv"):
            pipeline(bk_mm, bk_ew, (lambda g: []) if last else
                     (lambda g: preps((4, g - 1), *(
                         [] if isinstance(g, int) else [(5, g + 1), (6, g + 1)]))))
            _mix(bq_mm(0, 0), bk_ew(G - 1, 1), [] if last else preps((4, G - 1)))
        with jax.named_scope("b_q"):
            pipeline(bq_mm, bq_ew, (lambda g: []) if last else
                     (lambda g: preps((7, g - 1), *([(7, g)] * isinstance(g, int)))))
        with jax.named_scope("b_out"):
            if last:
                final_proj(bq_ew(G - 1, 1))
            else:
                out_proj(wbo, bq_ew(G - 1, 1), a_mm(0, 0))

    with jax.named_scope("wait_x"):
        start(xcopy + first)
        wait(xcopy + first)
        start(second + rest_a)
    with jax.named_scope("load_x"):
        _mix([functools.partial(load_x, r) for r in range(4)],
             preps((0, 0), (1, 0), (2, 0)))
        wait(second)
        for c in range(4):
            _mix(a_mm(0, 0)[3 * c:3 * c + 3],
                 [functools.partial(load_x, r) for r in range(4 * c + 4, R)][:4]
                 + preps(*[(k, 1) for k in range(3) if c == 3]))
        wait(rest_a)
        start(all_b)

    def a_prep(g):
        return preps(*([(k, g + 1) for k in range(3)] if not isinstance(g, int) else [(3, g)]),
                     (3, g - 1))

    for last in (False, True):
        with jax.named_scope("a_attn"):
            pipeline(a_mm, a_ew, (lambda g: []) if last else a_prep)
            if not last:
                wait(all_b)
        with jax.named_scope("a_out"):
                out_proj(wao, a_attn(G - 1, bufs[1], True), bk_mm(0, 0),
                     () if last else preps((5, 0), (6, 0), (5, 1), (6, 1)))
        layer_b(last)


@jax.jit
def pallas_interleave_layers__sliding_local_dilated__linear_kernel_hedgehog__prompt_kernel(
    A_x, A_wqkv, A_wo, B_x, B_wqkv, B_w_phi, B_wo):
    del B_x
    vmem = pltpu.VMEM
    out = pl.pallas_call(
        _kernel,
        grid=(1,),
        out_shape=jax.ShapeDtypeStruct((S, D), BF16),
        in_specs=[pl.BlockSpec(memory_space=pl.ANY)] * 6,
        out_specs=pl.BlockSpec(memory_space=pl.ANY),
        scratch_shapes=[
            vmem((G, S, T), BF16),
            vmem((8, D, D), BF16),
            vmem((D, DH), BF16),
            vmem((D, S), F32),
            vmem((D // 2, S), jnp.uint32),
            vmem((D // 2, S), jnp.uint32),
            vmem((G, 3 * T // 2, D), jnp.uint32),
            vmem((D // 2, D), jnp.uint32),
            vmem((G, 3 * T // 2, D), jnp.uint32),
            vmem((D // 2, D), jnp.uint32),
            vmem((3 * T, 2 * S), F32),
            vmem((3 * T, 2 * S), F32),
            vmem((T, S), jnp.uint32),
            vmem((T, S), jnp.uint32),
            vmem((G, T // 2 + 8, 2 * T), jnp.uint32),
            vmem((T + 16, 2 * T), F32),
            vmem((D, NC), F32), vmem((D, NC), F32),
            vmem((T, S), F32), vmem((T, S), F32),
            pltpu.SemaphoreType.DMA((6,)),
        ],
        compiler_params=pltpu.CompilerParams(
            vmem_limit_bytes=112 * 1024 * 1024),
    )(A_x.reshape(S, D), A_wqkv, A_wo, B_wqkv, B_w_phi.reshape(D, DH), B_wo)
    return out.reshape(1, S, D)
```

```python
import functools

import jax
import numpy as np
import jax.numpy as jnp
from jax import lax
import jax.experimental.pallas as pl
import jax.experimental.pallas.tpu as pltpu

S, D, H, DH, W, DIL = 2048, 1024, 32, 32, 8, 2
T = 128
R = S // T
G = D // T
NC = 512
F32, BF16 = jnp.float32, jnp.bfloat16
LOG2E = 1.4426950408889634
NT = (((1,), (1,)), ((), ()))


def _dot(a, b):
    return jnp.dot(a, b, preferred_element_type=F32)


def _rows(row, n):
    if isinstance(row, int):
        return pl.ds(row // 2, n // 2)
    return pl.ds(pl.multiple_of(row // 2, 8), n // 2)


def _ld(ref, g, row, n, cols=slice(None)):
    idx = (_rows(row, n), cols) if g is None else (g, _rows(row, n), cols)
    return pltpu.bitcast(ref[idx], BF16)


def _st(ref, g, row, cols, val):
    rows = _rows(row, val.shape[0])
    idx = (rows, cols) if g is None else (g, rows, cols)
    ref[idx] = pltpu.bitcast(val.astype(BF16), jnp.uint32)


def _mix0(*lists):
    items = [((i + 0.5) / len(l), j, f)
             for j, l in enumerate(lists) for i, f in enumerate(l)]
    for _, _, f in sorted(items, key=lambda t: t[:2]):
        f()


def _sub_allreduce(x, op):
    for d in (4, 2, 1):
        x = op(x, pltpu.roll(x, d, 0))
    return x


def _recip(s):
    r = pl.reciprocal(s, approx=True)
    return r * (2.0 - s * r)


def _fold4(x, op):
    return op(op(x[0:8], x[8:16]), op(x[16:24], x[24:32]))


def _normalize(x):
    m = jnp.sum(x.reshape(D // 8, 8, T), axis=0)
    m = _sub_allreduce(m, jnp.add) * (1.0 / D)
    c = x.reshape(D // 8, 8, T) - m
    v = _sub_allreduce(jnp.sum(c * c, axis=0), jnp.add) * (1.0 / D)
    return (c * lax.rsqrt(v + 1e-5)).reshape(D, T).astype(BF16)


def _kernel(x_hbm, awqkv_hbm, awo_hbm, bwqkv_hbm, phi_hbm, bwo_hbm, zeros_ref,
            out_hbm,
            xio, stage, phis, xt, xn, ot, ot7, wa, wao, wb, wbo, buf0, buf1,
            ph0, ph1, kvt, kvacc, y0, y1, yf0, yf1, sems):

    def wcopy(k, lo, n, sem):
        src = (awqkv_hbm, awqkv_hbm, awqkv_hbm, awo_hbm,
               bwqkv_hbm, bwqkv_hbm, bwqkv_hbm, bwo_hbm)[k]
        src = src.at[:, pl.ds((k % 4) * D * (k % 4 != 3) + lo, n)]
        return pltpu.make_async_copy(src, stage.at[k, :, pl.ds(lo, n)],
                                     sems.at[sem])

    xcopy = [pltpu.make_async_copy(x_hbm.at[:, pl.ds(j * T, T)], xio.at[j],
                                   sems.at[0]) for j in range(G)]
    first = [wcopy(k, 0, T, 1) for k in range(3)]
    second = [wcopy(k, T, T, 2) for k in range(3)]
    rest_a = [wcopy(k, 2 * T, D - 2 * T, 3) for k in range(3)]
    rest_a.append(wcopy(3, 0, D, 3))
    all_b = [wcopy(k, 0, D, 4) for k in range(4, 8)]
    all_b.append(pltpu.make_async_copy(phi_hbm, phis, sems.at[4]))

    def start(cps):
        for cp in cps:
            cp.start()

    def wait(cps):
        for cp in cps:
            cp.wait()

    xio32 = xio.bitcast(jnp.uint32)
    hi_mask = jnp.uint32(0xFFFF0000)

    def load_x(r):
        u = jnp.concatenate([xio32[j, pl.ds(r // 2, T, stride=R // 2), :]
                             for j in range(G)], axis=1)
        t = pltpu.bitcast((u & hi_mask) if r % 2 else (u << 16), F32).T
        cols = slice(r * T, (r + 1) * T)
        xt[:, cols] = t
        _st(xn, None, 0, cols, _normalize(t))

    def wt(k, g):
        c0 = g * T if isinstance(g, int) else pl.multiple_of(g * T, T)
        return stage[k, :, pl.ds(c0, T)].T

    def prep(k, g):
        dst, gi, row = (((wa, g, k * T),) * 3 + ((wao, None, g * T),)
                        + ((wb, g, k * T - 4 * T),) * 3 + ((wbo, None, g * T),))[k]
        w = wt(k, g)
        if k in (4, 5):
            r0 = g * T if isinstance(g, int) else pl.multiple_of(g * T, T)
            rows = phis[pl.ds(r0, T), :]
            bd = jnp.where(diag[:T, :T], jnp.concatenate([rows] * 4, axis=1), 0)
            w = _dot(bd.astype(F32).T.astype(BF16), w)
        _st(dst, gi, row, slice(None), w)

    def preps(*kg):
        return [functools.partial(prep, k, g) for k, g in kg]

    sub = lax.broadcasted_iota(jnp.int32, (8, T), 0)
    lane = lax.broadcasted_iota(jnp.int32, (8, T), 1)
    bufs = (buf0, buf1)
    ys, yf = (y0, y1), (yf0, yf1)
    phb = (ph0, ph1)

    def compact(ps):
        for d in (4, 2, 1):
            clear = (sub & d) == 0
            nxt = []
            for j in range(d):
                a, b = ps[j], ps[j + d]
                if d == 4:
                    nxt.append(jnp.where(clear, a, b)
                               + pltpu.roll(jnp.where(clear, b, a), 4, 0))
                else:
                    nxt.append(jnp.where(clear, a + pltpu.roll(a, 8 - d, 0),
                                         b + pltpu.roll(b, d, 0)))
            ps = nxt
        return ps[0]

    never = zeros_ref[...] != 0
    gate = [None, None]

    def mark(y):
        gate[:] = [gate[1], y[-8:, -T:]]

    def pace(x):
        if gate[0] is None:
            return x
        return jnp.where(never, gate[0], x.reshape(-1, 8, T)).reshape(x.shape)

    def _mix(*lists):
        gate[:] = [None, None]
        _mix0(*lists)
        gate[:] = [None, None]

    def put_o(g, h, cols, val):
        if isinstance(g, int) and g == G - 1:
            _st(ot7, None, h * DH, cols, val)
        else:
            _st(ot, None, g * T + h * DH, cols, val)

    def proj(w, g, row0, nblk, buf):
        def unit(k, c):
            cols = slice(c * NC, (c + 1) * NC)
            wk = _ld(w, g, row0 + k * T, T)
            y = _dot(wk, _ld(xn, None, 0, D, cols))
            buf[k * T:(k + 1) * T, cols] = y
            mark(y)
        return [functools.partial(unit, k, c)
                for c in range(S // NC) for k in range(nblk)]

    def a_attn(g, buf, tail=False):
        def shift(h):
            for sec in (1, 2):
                rows = slice(sec * T + h * DH, sec * T + (h + 1) * DH)
                for t in range(DIL, R):
                    buf[rows, (R + t) * T:(R + t + 1) * T] = pltpu.roll(
                        buf[rows, t * T:(t + 1) * T], 1, 1)

        def unit(h, r):
            def win(sec, w):
                t = (r - DIL * w) % (2 * R)
                return buf[sec * T + h * DH:sec * T + (h + 1) * DH,
                           t * T:(t + 1) * T]
            q = win(0, 0)
            lg = compact([_fold4(q * win(1, w), jnp.add) for w in range(W)])
            lg = lg * (DH ** -0.5)
            if r < DIL * (W - 1):
                lg = jnp.where((lane == 0) & (sub * DIL > r), -1e9, lg)
            e = jnp.exp(lg - _sub_allreduce(lg, jnp.maximum))
            p = e * _recip(_sub_allreduce(e, jnp.add))
            o = None
            for w in range(W):
                term = (win(2, w).reshape(DH // 8, 8, T)
                        * jnp.broadcast_to(p[w:w + 1], (8, T)))
                o = term if o is None else o + term
            put_o(g, h, slice(r * T, (r + 1) * T), o.reshape(DH, T))
        out = []
        if tail:
            return ([functools.partial(shift, h) for h in range(T // DH)]
                    + [functools.partial(unit, h, r)
                       for r in range(R) for h in range(T // DH)])
        for h in range(T // DH):
            out.append(functools.partial(shift, h))
            out += [functools.partial(unit, h, r) for r in reversed(range(R))]
        return out

    def pipeline(mm, ew, extra=lambda g: []):
        def body(i, _):
            _mix(mm(2 * i + 1, 1), ew(2 * i, 0), extra(2 * i + 1))
            _mix(mm(2 * i + 2, 0), ew(2 * i + 1, 1), extra(2 * i + 2))
        lax.fori_loop(0, G // 2 - 1, body, None)
        _mix(mm(G - 1, 1), ew(G - 2, 0), extra(G - 1))

    def wo_unit(wo, k, c, put, lo=0, hi=D):
        cols = slice(c * NC, (c + 1) * NC)
        y = None
        if lo == 0:
            y = _dot(_ld(wo, None, k * T, T, slice(0, D - T)),
                     _ld(ot, None, 0, D - T, cols))
        if hi == D:
            y7 = _dot(_ld(wo, None, k * T, T, slice(D - T, D)),
                      _ld(ot7, None, 0, T, cols))
            y = y7 if y is None else y + y7
        put(k, c, y)
        mark(y)

    def ln(c):
        def tile(r):
            cols = slice(r * T, (r + 1) * T)
            st = {}
            blk = lambda k: xt[k * T:(k + 1) * T, cols].reshape(T // 8, 8, T)

            def mean(k):
                x = (xt[k * T:(k + 1) * T, cols]
                     + ys[c % 2][k * T:(k + 1) * T, (r % n) * T:(r % n + 1) * T])
                if c == 0:
                    x = x + yf[k // 4][:, (k % 4 * n + r) * T:(k % 4 * n + r + 1) * T]
                xt[k * T:(k + 1) * T, cols] = x
                m = jnp.sum(pace(x).reshape(T // 8, 8, T), axis=0)
                st["m"] = m + st["m"] if k else m
                if k == G - 1:
                    st["m"] = _sub_allreduce(st["m"], jnp.add) * (1.0 / D)

            def var(k):
                d = blk(k) - pace(st["m"])
                v = jnp.sum(d * d, axis=0)
                st["v"] = v + st["v"] if k else v
                if k == G - 1:
                    v = _sub_allreduce(st["v"], jnp.add) * (1.0 / D)
                    st["v"] = lax.rsqrt(v + 1e-5)

            def norm(k):
                y = (blk(k) - pace(st["m"])) * st["v"]
                _st(xn, None, k * T, cols, y.reshape(T, T))
            return [functools.partial(f, k)
                    for f in (mean, var, norm) for k in range(G)]
        n = NC // T
        return [f for r in range(c * n, c * n + n) for f in tile(r)]

    def out_proj(wo, tail, nxt, extra=()):
        def put(k, c, y):
            ys[c % 2][k * T:(k + 1) * T, :] = y
        def add(k, c, y):
            yf[k // 4][:, (k % 4) * NC:(k % 4 + 1) * NC] = y
        mm = lambda c, f=put, lo=0, hi=D: [
            functools.partial(wo_unit, wo, k, c, f, lo, hi) for k in range(G)]
        _mix(mm(0, put, 0, D - T), tail)
        _mix(mm(0, add, D - T, D))
        for c in range(1, S // NC):
            _mix(mm(c), ln(c - 1), extra[c - 1::3])
        _mix(nxt[:len(nxt) // 2], ln(S // NC - 1))
        _mix(nxt[len(nxt) // 2:])

    a_mm = lambda g, s: proj(wa, g, 0, 3, bufs[s])
    a_ew = lambda g, s: a_attn(g, bufs[s])
    bk_mm = lambda g, s: proj(wb, g, T, 2, bufs[s])
    bq_mm = lambda g, s: proj(wb, g, 0, 1, bufs[s])

    def feature_map(paced, src, dst, c):
        def unit(h, r):
            cols = slice(r * T, (r + 1) * T)
            p = src[h * DH:(h + 1) * DH, cols] * LOG2E
            if paced:
                p = pace(p)
            for sgn, op in ((0, jnp.maximum), (1, jnp.minimum)):
                m = _sub_allreduce(_fold4(p, op), op)
                p3 = p.reshape(DH // 8, 8, T)
                e = jnp.exp2(m - p3 if sgn else p3 - m)
                inv = _recip(_sub_allreduce(jnp.sum(e, axis=0), jnp.add))
                _st(dst, None, sgn * T + h * DH, cols, (e * inv).reshape(DH, T))
        n = NC // T
        return [functools.partial(unit, h, r)
                for r in range(c * n, c * n + n) for h in range(T // DH)]

    rowh = lax.broadcasted_iota(jnp.int32, (T + 16, 2 * T), 0)
    colh = (lax.broadcasted_iota(jnp.int32, (T + 16, 2 * T), 1) % T) // DH
    diag = jnp.where(rowh < T, rowh // DH, rowh - T) == colh

    def skew(fm, mm):
        out = []
        for c in range(S // NC):
            f = fm(c)
            out += f[:2]
            if c:
                out.append(functools.partial(mm, c - 1))
            out += f[2:]
        return out + [functools.partial(mm, S // NC - 1)]

    def bk_ew(g, s):
        buf, ph = bufs[s], phb[s]

        def mm(c):
            cols = slice(c * NC, (c + 1) * NC)
            v = jnp.concatenate([buf[T:2 * T, cols].astype(BF16),
                                 jnp.ones((16, NC), BF16)], axis=0)
            kv = lax.dot_general(v, _ld(ph, None, 0, 2 * T, cols), NT,
                                 preferred_element_type=F32)
            if c:
                kv = kv + kvacc[...]
            if c < S // NC - 1:
                kvacc[...] = kv
            else:
                _st(kvt, g, 0, slice(None), jnp.where(diag, kv, 0.0))
        return skew(functools.partial(feature_map, not isinstance(g, int) or g < G - 1, buf, ph), mm)

    def bq_ew(g, s):
        buf, ph = bufs[s], phb[s]

        def mm(c):
            cols = slice(c * NC, (c + 1) * NC)
            nd = _dot(_ld(kvt, g, 0, T + 16), _ld(ph, None, 0, 2 * T, cols))
            inv = 1.0 / (nd[T:T + 8] + 1e-6)
            for h in range(T // DH):
                put_o(g, h, cols, nd[h * DH:(h + 1) * DH] * inv[h:h + 1])
        return skew(functools.partial(feature_map, False, buf, ph), mm)

    def store(j, src):
        def unit(m):
            def bits(r):
                t = xt[_rows(2 * j * T, 2 * T), r * T:(r + 1) * T]
                t = t + src[:, r * T:(r + 1) * T]
                return pltpu.bitcast(t.astype(BF16).astype(F32).T, jnp.uint32)
            xio32[j, pl.ds(m, T, stride=R // 2), :] = (
                (bits(2 * m) >> 16) | bits(2 * m + 1))
        return [functools.partial(unit, m) for m in range(R // 2)]

    def ocopy(j):
        c0 = j * T if isinstance(j, int) else pl.multiple_of(j * T, T)
        return pltpu.make_async_copy(xio.at[j], out_hbm.at[:, pl.ds(c0, T)],
                                     sems.at[5])

    def final_proj(tail):
        def mm(k, s, lo=0, hi=D):
            def put(k, c, y):
                if lo:
                    y = y + yf[s][:, c * NC:(c + 1) * NC]
                yf[s][:, c * NC:(c + 1) * NC] = y
            return [functools.partial(wo_unit, wbo, k, c, put, lo, hi)
                    for c in range(S // NC)]
        _mix(mm(0, 0, 0, D - T), tail)
        _mix(mm(0, 0, D - T, D))
        _mix(mm(1, 1), store(0, yf[0]))

        def body(i, _):
            ocopy(2 * i - 2).start()
            _mix(mm(2 * i, 0), store(2 * i - 1, yf[1]))
            _mix(mm(2 * i + 1, 1), store(2 * i, yf[0]))

            @pl.when(pl.program_id(0) == 0)
            def _():
                ocopy(2 * i - 1).start()
        lax.fori_loop(1, G // 2, body, None)
        ocopy(G - 2).start()
        _mix(store(G - 1, yf[1]))
        pl.when(pl.program_id(0) == 0)(ocopy(G - 1).start)
        wait([ocopy(k) for k in range(G)])

    def layer_b(last):
        with jax.named_scope("b_kv"):
            pipeline(bk_mm, bk_ew, (lambda g: []) if last else
                     (lambda g: preps((4, g - 1), *(
                         [] if isinstance(g, int) else [(5, g + 1), (6, g + 1)]))))
            _mix(bq_mm(0, 0), bk_ew(G - 1, 1), [] if last else preps((4, G - 1)))
        with jax.named_scope("b_q"):
            pipeline(bq_mm, bq_ew, (lambda g: []) if last else
                     (lambda g: preps((7, g - 1), *([(7, g)] * isinstance(g, int)))))
        with jax.named_scope("b_out"):
            if last:
                final_proj(bq_ew(G - 1, 1))
            else:
                out_proj(wbo, bq_ew(G - 1, 1), a_mm(0, 0))

    with jax.named_scope("wait_x"):
        start(xcopy + first)
        wait(xcopy + first)
        start(second + rest_a)
    with jax.named_scope("load_x"):
        _mix([functools.partial(load_x, r) for r in range(4)],
             preps((0, 0), (1, 0), (2, 0)))
        wait(second)
        for c in range(4):
            _mix(a_mm(0, 0)[3 * c:3 * c + 3],
                 [functools.partial(load_x, r) for r in range(4 * c + 4, R)][:4]
                 + preps(*[(k, 1) for k in range(3) if c == 3]))
        wait(rest_a)
        start(all_b)

    def a_prep(g):
        return preps(*([(k, g + 1) for k in range(3)] if not isinstance(g, int) else [(3, g)]),
                     (3, g - 1))

    for last in (False, True):
        with jax.named_scope("a_attn"):
            pipeline(a_mm, a_ew, (lambda g: []) if last else a_prep)
            if not last:
                wait(all_b)
        with jax.named_scope("a_out"):
                out_proj(wao, a_attn(G - 1, bufs[1], True), bk_mm(0, 0),
                     () if last else preps((5, 0), (6, 0), (5, 1), (6, 1)))
        layer_b(last)


@jax.jit
def pallas_interleave_layers__sliding_local_dilated__linear_kernel_hedgehog__prompt_kernel(
    A_x, A_wqkv, A_wo, B_x, B_wqkv, B_w_phi, B_wo):
    del B_x
    vmem = pltpu.VMEM
    out = pl.pallas_call(
        _kernel,
        grid=(1,),
        out_shape=jax.ShapeDtypeStruct((S, D), BF16),
        in_specs=[pl.BlockSpec(memory_space=pl.ANY)] * 6
        + [pl.BlockSpec((8, T), lambda i: (0, 0))],
        out_specs=pl.BlockSpec(memory_space=pl.ANY),
        scratch_shapes=[
            vmem((G, S, T), BF16),
            vmem((8, D, D), BF16),
            vmem((D, DH), BF16),
            vmem((D, S), F32),
            vmem((D // 2, S), jnp.uint32),
            vmem(((D - T) // 2, S), jnp.uint32),
            vmem((T // 2, S), jnp.uint32),
            vmem((G, 3 * T // 2, D), jnp.uint32),
            vmem((D // 2, D), jnp.uint32),
            vmem((G, 3 * T // 2, D), jnp.uint32),
            vmem((D // 2, D), jnp.uint32),
            vmem((3 * T, 2 * S), F32),
            vmem((3 * T, 2 * S), F32),
            vmem((T, S), jnp.uint32),
            vmem((T, S), jnp.uint32),
            vmem((G, T // 2 + 8, 2 * T), jnp.uint32),
            vmem((T + 16, 2 * T), F32),
            vmem((D, NC), F32), vmem((D, NC), F32),
            vmem((T, S), F32), vmem((T, S), F32),
            pltpu.SemaphoreType.DMA((6,)),
        ],
        compiler_params=pltpu.CompilerParams(
            vmem_limit_bytes=112 * 1024 * 1024),
    )(A_x.reshape(S, D), A_wqkv, A_wo, B_wqkv, B_w_phi.reshape(D, DH), B_wo,
      np.zeros((8, T), np.int32))
    return out.reshape(1, S, D)
```

```python
import functools

import jax
import numpy as np
import jax.numpy as jnp
from jax import lax
import jax.experimental.pallas as pl
import jax.experimental.pallas.tpu as pltpu

S, D, H, DH, W, DIL = 2048, 1024, 32, 32, 8, 2
T = 128
R = S // T
G = D // T
NC = 512
F32, BF16 = jnp.float32, jnp.bfloat16
LOG2E = 1.4426950408889634
NT = (((1,), (1,)), ((), ()))


def _dot(a, b):
    return jnp.dot(a, b, preferred_element_type=F32)


def _rows(row, n):
    if isinstance(row, int):
        return pl.ds(row // 2, n // 2)
    return pl.ds(pl.multiple_of(row // 2, 8), n // 2)


def _ld(ref, g, row, n, cols=slice(None)):
    idx = (_rows(row, n), cols) if g is None else (g, _rows(row, n), cols)
    return pltpu.bitcast(ref[idx], BF16)


def _st(ref, g, row, cols, val):
    rows = _rows(row, val.shape[0])
    idx = (rows, cols) if g is None else (g, rows, cols)
    ref[idx] = pltpu.bitcast(val.astype(BF16), jnp.uint32)


def _mix0(*lists):
    items = [((i + 0.5) / len(l), j, f)
             for j, l in enumerate(lists) for i, f in enumerate(l)]
    for _, _, f in sorted(items, key=lambda t: t[:2]):
        f()


def _sub_allreduce(x, op):
    for d in (4, 2, 1):
        x = op(x, pltpu.roll(x, d, 0))
    return x


def _recip(s):
    r = pl.reciprocal(s, approx=True)
    return r * (2.0 - s * r)


def _fold4(x, op):
    return op(op(x[0:8], x[8:16]), op(x[16:24], x[24:32]))


def _kernel(x_hbm, awqkv_hbm, awo_hbm, bwqkv_hbm, phi_hbm, bwo_hbm, zeros_hbm,
            out_hbm,
            xio, stage, phis, xt, xn, ot, ot7, wa, wao, wb, wbo, buf0, buf1,
            ph0, ph1, kvt, kvacc, y0, y1, yf0, yf1, zeros_ref, sems):

    def wcopy(k, lo, n, sem):
        src = (awqkv_hbm, awqkv_hbm, awqkv_hbm, awo_hbm,
               bwqkv_hbm, bwqkv_hbm, bwqkv_hbm, bwo_hbm)[k]
        src = src.at[:, pl.ds((k % 4) * D * (k % 4 != 3) + lo, n)]
        return pltpu.make_async_copy(src, stage.at[k, :, pl.ds(lo, n)],
                                     sems.at[sem])

    xcopy = [pltpu.make_async_copy(x_hbm.at[:, pl.ds(j * T, T)], xio.at[j],
                                   sems.at[7 + j]) for j in range(G)]
    first = [wcopy(k, 0, T, 1) for k in range(3)]
    second = [wcopy(k, T, T, 2) for k in range(3)]
    first.append(pltpu.make_async_copy(zeros_hbm, zeros_ref, sems.at[1]))
    second += [wcopy(k, 2 * T, 2 * T, 2) for k in range(3)]
    second.append(wcopy(3, 0, 2 * T, 2))
    rest_a = [wcopy(k, 4 * T, D - 4 * T, 3) for k in range(3)]
    rest_a.append(wcopy(3, 2 * T, D - 2 * T, 3))
    all_b = [wcopy(k, 0, D, 4) for k in range(4, 8)]
    all_b.append(pltpu.make_async_copy(phi_hbm, phis, sems.at[4]))

    def start(cps):
        for cp in cps:
            cp.start()

    def wait(cps):
        for cp in cps:
            cp.wait()

    xio32 = xio.bitcast(jnp.uint32)
    hi_mask = jnp.uint32(0xFFFF0000)

    def load_x(j):
        for m in range(R // 2):
            u = xio32[j, pl.ds(m, T, stride=R // 2), :].T
            for par, bits in enumerate((u << 16, u & hi_mask)):
                r = 2 * m + par
                xt[j * T:(j + 1) * T, r * T:(r + 1) * T] = pltpu.bitcast(bits, F32)

    def wt(k, g):
        c0 = g * T if isinstance(g, int) else pl.multiple_of(g * T, T)
        return stage[k, :, pl.ds(c0, T)].T

    def prep(k, g):
        dst, gi, row = (((wa, g, k * T),) * 3 + ((wao, None, g * T),)
                        + ((wb, g, k * T - 4 * T),) * 3 + ((wbo, None, g * T),))[k]
        w = wt(k, g)
        if k in (4, 5):
            r0 = g * T if isinstance(g, int) else pl.multiple_of(g * T, T)
            rows = phis[pl.ds(r0, T), :]
            bd = jnp.where(diag[:T, :T], jnp.concatenate([rows] * 4, axis=1), 0)
            w = _dot(bd.astype(F32).T.astype(BF16), w)
        _st(dst, gi, row, slice(None), w)

    def preps(*kg):
        return [functools.partial(prep, k, g) for k, g in kg]

    sub = lax.broadcasted_iota(jnp.int32, (8, T), 0)
    lane = lax.broadcasted_iota(jnp.int32, (8, T), 1)
    bufs = (buf0, buf1)
    ys, yf = (y0, y1), (yf0, yf1)
    phb = (ph0, ph1)

    def compact(ps):
        for d in (4, 2, 1):
            clear = (sub & d) == 0
            nxt = []
            for j in range(d):
                a, b = ps[j], ps[j + d]
                if d == 4:
                    nxt.append(jnp.where(clear, a, b)
                               + pltpu.roll(jnp.where(clear, b, a), 4, 0))
                else:
                    nxt.append(jnp.where(clear, a + pltpu.roll(a, 8 - d, 0),
                                         b + pltpu.roll(b, d, 0)))
            ps = nxt
        return ps[0]

    gate = [None, None]

    def mark(y):
        gate[:] = [gate[1], y[-8:, -T:]]

    def pace(x):
        if gate[0] is None:
            return x
        return jnp.where(zeros_ref[...] != 0, gate[0], x.reshape(-1, 8, T)).reshape(x.shape)

    def _mix(*lists):
        gate[:] = [None, None]
        _mix0(*lists)
        gate[:] = [None, None]

    def put_o(g, h, cols, val):
        if isinstance(g, int) and g == G - 1:
            _st(ot7, None, h * DH, cols, val)
        else:
            _st(ot, None, g * T + h * DH, cols, val)

    def proj(w, g, row0, nblk, buf):
        def unit(k, c):
            cols = slice(c * NC, (c + 1) * NC)
            wk = _ld(w, g, row0 + k * T, T)
            y = _dot(wk, _ld(xn, None, 0, D, cols))
            buf[k * T:(k + 1) * T, cols] = y
            mark(y)
        return [functools.partial(unit, k, c)
                for c in range(S // NC) for k in range(nblk)]

    def a_attn(g, buf, tail=False):
        def shift(h):
            for sec in (1, 2):
                rows = slice(sec * T + h * DH, sec * T + (h + 1) * DH)
                for t in range(DIL, R):
                    buf[rows, (R + t) * T:(R + t + 1) * T] = pltpu.roll(
                        buf[rows, t * T:(t + 1) * T], 1, 1)

        def unit(h, r):
            def win(sec, w):
                t = (r - DIL * w) % (2 * R)
                return buf[sec * T + h * DH:sec * T + (h + 1) * DH,
                           t * T:(t + 1) * T]
            q = win(0, 0)
            lg = compact([_fold4(q * win(1, w), jnp.add) for w in range(W)])
            lg = lg * (DH ** -0.5)
            if r < DIL * (W - 1):
                lg = jnp.where((lane == 0) & (sub * DIL > r), -1e9, lg)
            e = jnp.exp(lg - _sub_allreduce(lg, jnp.maximum))
            p = e * _recip(_sub_allreduce(e, jnp.add))
            o = None
            for w in range(W):
                term = (win(2, w).reshape(DH // 8, 8, T)
                        * jnp.broadcast_to(p[w:w + 1], (8, T)))
                o = term if o is None else o + term
            put_o(g, h, slice(r * T, (r + 1) * T), o.reshape(DH, T))
        out = []
        if tail:
            return ([functools.partial(shift, h) for h in range(T // DH)]
                    + [functools.partial(unit, h, r)
                       for r in range(R) for h in range(T // DH)])
        for h in range(T // DH):
            out.append(functools.partial(shift, h))
            out += [functools.partial(unit, h, r) for r in reversed(range(R))]
        return out

    def pipeline(mm, ew, extra=lambda g: [], top=None):
        def body(i, _):
            if top:
                pl.when(i == 1)(top)
            _mix(mm(2 * i + 1, 1), ew(2 * i, 0), extra(2 * i + 1))
            _mix(mm(2 * i + 2, 0), ew(2 * i + 1, 1), extra(2 * i + 2))
        lax.fori_loop(0, G // 2 - 1, body, None)
        _mix(mm(G - 1, 1), ew(G - 2, 0), extra(G - 1))

    def wo_unit(wo, k, c, put, lo=0, hi=D):
        cols = slice(c * NC, (c + 1) * NC)
        y = None
        if lo == 0:
            y = _dot(_ld(wo, None, k * T, T, slice(0, D - T)),
                     _ld(ot, None, 0, D - T, cols))
        if hi == D:
            y7 = _dot(_ld(wo, None, k * T, T, slice(D - T, D)),
                      _ld(ot7, None, 0, T, cols))
            y = y7 if y is None else y + y7
        put(k, c, y)
        mark(y)

    def ln(c, add=True):
        def tile(r):
            cols = slice(r * T, (r + 1) * T)
            st = {}
            blk = lambda k: xt[k * T:(k + 1) * T, cols].reshape(T // 8, 8, T)

            def mean(k):
                x = xt[k * T:(k + 1) * T, cols]
                if add:
                    x = x + ys[c % 2][k * T:(k + 1) * T, (r % n) * T:(r % n + 1) * T]
                    if c == 0:
                        x = x + yf[k // 4][:, (k % 4 * n + r) * T:(k % 4 * n + r + 1) * T]
                    xt[k * T:(k + 1) * T, cols] = x
                m = jnp.sum(pace(x).reshape(T // 8, 8, T), axis=0)
                st["m"] = m + st["m"] if k else m
                if k == G - 1:
                    st["m"] = _sub_allreduce(st["m"], jnp.add) * (1.0 / D)

            def var(k):
                d = blk(k) - pace(st["m"])
                v = jnp.sum(d * d, axis=0)
                st["v"] = v + st["v"] if k else v
                if k == G - 1:
                    v = _sub_allreduce(st["v"], jnp.add) * (1.0 / D)
                    st["v"] = lax.rsqrt(v + 1e-5)

            def norm(k):
                y = (blk(k) - pace(st["m"])) * st["v"]
                _st(xn, None, k * T, cols, y.reshape(T, T))
            return [functools.partial(f, k)
                    for f in (mean, var, norm) for k in range(G)]
        n = NC // T
        return [f for r in range(c * n, c * n + n) for f in tile(r)]

    def out_proj(wo, tail, nxt, extra=()):
        def put(k, c, y):
            ys[c % 2][k * T:(k + 1) * T, :] = y
        def add(k, c, y):
            yf[k // 4][:, (k % 4) * NC:(k % 4 + 1) * NC] = y
        mm = lambda c, f=put, lo=0, hi=D: [
            functools.partial(wo_unit, wo, k, c, f, lo, hi) for k in range(G)]
        _mix(mm(0, put, 0, D - T), tail)
        _mix(mm(0, add, D - T, D))
        for c in range(1, S // NC):
            _mix(mm(c), ln(c - 1), extra[c - 1::3])
        _mix(nxt[:len(nxt) // 2], ln(S // NC - 1))
        _mix(nxt[len(nxt) // 2:])

    a_mm = lambda g, s: proj(wa, g, 0, 3, bufs[s])
    a_ew = lambda g, s: a_attn(g, bufs[s])
    bk_mm = lambda g, s: proj(wb, g, T, 2, bufs[s])
    bq_mm = lambda g, s: proj(wb, g, 0, 1, bufs[s])

    def feature_map(paced, src, dst, c):
        def unit(h, r):
            cols = slice(r * T, (r + 1) * T)
            p = src[h * DH:(h + 1) * DH, cols] * LOG2E
            if paced:
                p = pace(p)
            for sgn, op in ((0, jnp.maximum), (1, jnp.minimum)):
                m = _sub_allreduce(_fold4(p, op), op)
                p3 = p.reshape(DH // 8, 8, T)
                e = jnp.exp2(m - p3 if sgn else p3 - m)
                inv = _recip(_sub_allreduce(jnp.sum(e, axis=0), jnp.add))
                _st(dst, None, sgn * T + h * DH, cols, (e * inv).reshape(DH, T))
        n = NC // T
        return [functools.partial(unit, h, r)
                for r in range(c * n, c * n + n) for h in range(T // DH)]

    rowh = lax.broadcasted_iota(jnp.int32, (T + 16, 2 * T), 0)
    colh = (lax.broadcasted_iota(jnp.int32, (T + 16, 2 * T), 1) % T) // DH
    diag = jnp.where(rowh < T, rowh // DH, rowh - T) == colh

    def skew(fm, mm):
        out = []
        for c in range(S // NC):
            f = fm(c)
            out += f[:2]
            if c:
                out.append(functools.partial(mm, c - 1))
            out += f[2:]
        return out + [functools.partial(mm, S // NC - 1)]

    def bk_ew(g, s):
        buf, ph = bufs[s], phb[s]

        def mm(c):
            cols = slice(c * NC, (c + 1) * NC)
            v = jnp.concatenate([buf[T:2 * T, cols].astype(BF16),
                                 jnp.ones((16, NC), BF16)], axis=0)
            kv = lax.dot_general(v, _ld(ph, None, 0, 2 * T, cols), NT,
                                 preferred_element_type=F32)
            if c:
                kv = kv + kvacc[...]
            if c < S // NC - 1:
                kvacc[...] = kv
            else:
                _st(kvt, g, 0, slice(None), jnp.where(diag, kv, 0.0))
        return skew(functools.partial(feature_map, not isinstance(g, int) or g < G - 1, buf, ph), mm)

    def bq_ew(g, s):
        buf, ph = bufs[s], phb[s]

        def mm(c):
            cols = slice(c * NC, (c + 1) * NC)
            nd = _dot(_ld(kvt, g, 0, T + 16), _ld(ph, None, 0, 2 * T, cols))
            inv = 1.0 / (nd[T:T + 8] + 1e-6)
            for h in range(T // DH):
                put_o(g, h, cols, nd[h * DH:(h + 1) * DH] * inv[h:h + 1])
        return skew(functools.partial(feature_map, False, buf, ph), mm)

    def store(j, src):
        def unit(m):
            def bits(r):
                t = xt[_rows(2 * j * T, 2 * T), r * T:(r + 1) * T]
                t = t + src[:, r * T:(r + 1) * T]
                return pltpu.bitcast(t.astype(BF16).astype(F32), jnp.uint32)
            xio32[j, pl.ds(m, T, stride=R // 2), :] = (
                (bits(2 * m) >> 16) | bits(2 * m + 1)).T
        return [functools.partial(unit, m) for m in range(R // 2)]

    def ocopy(j):
        c0 = j * T if isinstance(j, int) else pl.multiple_of(j * T, T)
        return pltpu.make_async_copy(xio.at[j], out_hbm.at[:, pl.ds(c0, T)],
                                     sems.at[5])

    def final_proj(tail):
        def mm(k, s, lo=0, hi=D):
            def put(k, c, y):
                if lo:
                    y = y + yf[s][:, c * NC:(c + 1) * NC]
                yf[s][:, c * NC:(c + 1) * NC] = y
            return [functools.partial(wo_unit, wbo, k, c, put, lo, hi)
                    for c in range(S // NC)]
        _mix(mm(0, 0, 0, D - T), tail)
        _mix(mm(0, 0, D - T, D))
        _mix(mm(1, 1), store(0, yf[0]))

        def body(i, _):
            ocopy(2 * i - 2).start()
            _mix(mm(2 * i, 0), store(2 * i - 1, yf[1]))
            _mix(mm(2 * i + 1, 1), store(2 * i, yf[0]))

            @pl.when(pl.program_id(0) == 0)
            def _():
                ocopy(2 * i - 1).start()
        lax.fori_loop(1, G // 2, body, None)
        ocopy(G - 2).start()
        _mix(store(G - 1, yf[1]))
        pl.when(pl.program_id(0) == 0)(ocopy(G - 1).start)
        wait([ocopy(k) for k in range(G)])

    def layer_b(last):
        with jax.named_scope("b_kv"):
            pipeline(bk_mm, bk_ew, (lambda g: []) if last else
                     (lambda g: preps((4, g - 1), *(
                         [] if isinstance(g, int) else [(5, g + 1), (6, g + 1)]))))
            _mix(bq_mm(0, 0), bk_ew(G - 1, 1), [] if last else preps((4, G - 1)))
        with jax.named_scope("b_q"):
            pipeline(bq_mm, bq_ew, (lambda g: []) if last else
                     (lambda g: preps((7, g - 1), *([(7, g)] * isinstance(g, int)))))
        with jax.named_scope("b_out"):
            if last:
                final_proj(bq_ew(G - 1, 1))
            else:
                out_proj(wbo, bq_ew(G - 1, 1), a_mm(0, 0))

    with jax.named_scope("load_x"):
        issue = [[cp] for cp in xcopy] + [[], [], second]
        start(first + issue[0] + issue[1] + issue[2])
        for j in range(G):
            wait(issue[j])
            start(issue[j + 3])
            load_x(j)
            if j == 0:
                wait(first)
                _mix(preps((0, 0), (1, 0), (2, 0)))
        _mix(ln(0, False))
        for c in range(4):
            if c == 2:
                wait(second)
                start(rest_a)
            _mix(a_mm(0, 0)[3 * c:3 * c + 3],
                 ln(c + 1, False) if c < 3 else preps((0, 1), (1, 1), (2, 1)))

    def a_prep(g):
        return preps(*([(k, g + 1) for k in range(3)] if not isinstance(g, int) else [(3, g)]),
                     (3, g - 1))

    for last in (False, True):
        with jax.named_scope("a_attn"):
            if last:
                pipeline(a_mm, a_ew)
            else:
                pipeline(a_mm, a_ew, a_prep,
                         lambda: (wait(rest_a), start(all_b)) and None)
            if not last:
                wait(all_b)
        with jax.named_scope("a_out"):
                out_proj(wao, a_attn(G - 1, bufs[1], True), bk_mm(0, 0),
                     () if last else preps((5, 0), (6, 0), (5, 1), (6, 1)))
        layer_b(last)


@jax.jit
def pallas_interleave_layers__sliding_local_dilated__linear_kernel_hedgehog__prompt_kernel(
    A_x, A_wqkv, A_wo, B_x, B_wqkv, B_w_phi, B_wo):
    del B_x
    vmem = pltpu.VMEM
    out = pl.pallas_call(
        _kernel,
        grid=(1,),
        out_shape=jax.ShapeDtypeStruct((S, D), BF16),
        in_specs=[pl.BlockSpec(memory_space=pl.ANY)] * 7,
        out_specs=pl.BlockSpec(memory_space=pl.ANY),
        scratch_shapes=[
            vmem((G, S, T), BF16),
            vmem((8, D, D), BF16),
            vmem((D, DH), BF16),
            vmem((D, S), F32),
            vmem((D // 2, S), jnp.uint32),
            vmem(((D - T) // 2, S), jnp.uint32),
            vmem((T // 2, S), jnp.uint32),
            vmem((G, 3 * T // 2, D), jnp.uint32),
            vmem((D // 2, D), jnp.uint32),
            vmem((G, 3 * T // 2, D), jnp.uint32),
            vmem((D // 2, D), jnp.uint32),
            vmem((3 * T, 2 * S), F32),
            vmem((3 * T, 2 * S), F32),
            vmem((T, S), jnp.uint32),
            vmem((T, S), jnp.uint32),
            vmem((G, T // 2 + 8, 2 * T), jnp.uint32),
            vmem((T + 16, 2 * T), F32),
            vmem((D, NC), F32), vmem((D, NC), F32),
            vmem((T, S), F32), vmem((T, S), F32),
            vmem((8, T), jnp.int32),
            pltpu.SemaphoreType.DMA((7 + G,)),
        ],
        compiler_params=pltpu.CompilerParams(
            vmem_limit_bytes=112 * 1024 * 1024),
    )(A_x.reshape(S, D), A_wqkv, A_wo, B_wqkv, B_w_phi.reshape(D, DH), B_wo,
      np.zeros((8, T), np.int32))
    return out.reshape(1, S, D)
```

```python
import functools

import jax
import numpy as np
import jax.numpy as jnp
from jax import lax
import jax.experimental.pallas as pl
import jax.experimental.pallas.tpu as pltpu

S, D, H, DH, W, DIL = 2048, 1024, 32, 32, 8, 2
T = 128
R = S // T
G = D // T
NC = 512
F32, BF16 = jnp.float32, jnp.bfloat16
LOG2E = 1.4426950408889634
NT = (((1,), (1,)), ((), ()))


def _dot(a, b):
    return jnp.dot(a, b, preferred_element_type=F32)


def _rows(row, n):
    if isinstance(row, int):
        return pl.ds(row // 2, n // 2)
    return pl.ds(pl.multiple_of(row // 2, 8), n // 2)


def _ld(ref, g, row, n, cols=slice(None)):
    idx = (_rows(row, n), cols) if g is None else (g, _rows(row, n), cols)
    return pltpu.bitcast(ref[idx], BF16)


def _st(ref, g, row, cols, val):
    rows = _rows(row, val.shape[0])
    idx = (rows, cols) if g is None else (g, rows, cols)
    ref[idx] = pltpu.bitcast(val.astype(BF16), jnp.uint32)


def _mix0(*lists):
    items = [((i + 0.5) / len(l), j, f)
             for j, l in enumerate(lists) for i, f in enumerate(l)]
    for _, _, f in sorted(items, key=lambda t: t[:2]):
        f()


def _sub_allreduce(x, op):
    for d in (4, 2, 1):
        x = op(x, pltpu.roll(x, d, 0))
    return x


def _recip(s):
    r = pl.reciprocal(s, approx=True)
    return r * (2.0 - s * r)


def _fold4(x, op):
    return op(op(x[0:8], x[8:16]), op(x[16:24], x[24:32]))


def _kernel(x_hbm, awqkv_hbm, awo_hbm, bwqkv_hbm, phi_hbm, bwo_hbm, zeros_hbm,
            out_hbm,
            xio, stage, phis, xt, xn, ot, ot7, wa, wao, wb, wbo, buf0, buf1,
            ph0, ph1, kvt, kvacc, y0, y1, yf0, yf1, zeros_ref, sems):

    def wcopy(k, lo, n, sem):
        src = (awqkv_hbm, awqkv_hbm, awqkv_hbm, awo_hbm,
               bwqkv_hbm, bwqkv_hbm, bwqkv_hbm, bwo_hbm)[k]
        src = src.at[:, pl.ds((k % 4) * D * (k % 4 != 3) + lo, n)]
        return pltpu.make_async_copy(src, stage.at[k, :, pl.ds(lo, n)],
                                     sems.at[sem])

    xcopy = [pltpu.make_async_copy(x_hbm.at[:, pl.ds(j * T, T)], xio.at[j],
                                   sems.at[7 + j]) for j in range(G)]
    first = [wcopy(k, 0, T, 1) for k in range(3)]
    second = [wcopy(k, T, T, 2) for k in range(3)]
    first.append(pltpu.make_async_copy(zeros_hbm, zeros_ref, sems.at[1]))
    second += [wcopy(k, 2 * T, 2 * T, 2) for k in range(3)]
    second.append(wcopy(3, 0, 2 * T, 2))
    rest_a = [wcopy(k, 4 * T, D - 4 * T, 3) for k in range(3)]
    rest_a.append(wcopy(3, 2 * T, D - 2 * T, 3))
    all_b = [wcopy(k, 0, D, 4) for k in range(4, 8)]
    all_b.append(pltpu.make_async_copy(phi_hbm, phis, sems.at[4]))

    def start(cps):
        for cp in cps:
            cp.start()

    def wait(cps):
        for cp in cps:
            cp.wait()

    xio32 = xio.bitcast(jnp.uint32)
    hi_mask = jnp.uint32(0xFFFF0000)

    def load_x(j):
        for m in range(R // 2):
            u = xio32[j, pl.ds(m, T, stride=R // 2), :].T
            for par, bits in enumerate((u << 16, u & hi_mask)):
                r = 2 * m + par
                xt[j * T:(j + 1) * T, r * T:(r + 1) * T] = pltpu.bitcast(bits, F32)

    def wt(k, g):
        c0 = g * T if isinstance(g, int) else pl.multiple_of(g * T, T)
        return stage[k, :, pl.ds(c0, T)].T

    def prep(k, g):
        dst, gi, row = (((wa, g, k * T),) * 3 + ((wao, None, g * T),)
                        + ((wb, g, k * T - 4 * T),) * 3 + ((wbo, None, g * T),))[k]
        w = wt(k, g)
        if k in (4, 5):
            r0 = g * T if isinstance(g, int) else pl.multiple_of(g * T, T)
            rows = phis[pl.ds(r0, T), :]
            bd = jnp.where(phi_diag, jnp.concatenate([rows] * 4, axis=1), 0)
            w = _dot(bd.astype(F32).T.astype(BF16), w)
        _st(dst, gi, row, slice(None), w)

    def preps(*kg):
        return [functools.partial(prep, k, g) for k, g in kg]

    sub = lax.broadcasted_iota(jnp.int32, (8, T), 0)
    lane = lax.broadcasted_iota(jnp.int32, (8, T), 1)
    bufs = (buf0, buf1)
    ys, yf = (y0, y1), (yf0, yf1)
    phb = (ph0, ph1)

    def compact(ps):
        for d in (4, 2, 1):
            clear = (sub & d) == 0
            nxt = []
            for j in range(d):
                a, b = ps[j], ps[j + d]
                if d == 4:
                    nxt.append(jnp.where(clear, a, b)
                               + pltpu.roll(jnp.where(clear, b, a), 4, 0))
                else:
                    nxt.append(jnp.where(clear, a + pltpu.roll(a, 8 - d, 0),
                                         b + pltpu.roll(b, d, 0)))
            ps = nxt
        return ps[0]

    gate = [None, None]

    def mark(y):
        gate[:] = [gate[1], y[-8:, -T:]]

    def pace(x):
        if gate[0] is None:
            return x
        return jnp.where(zeros_ref[...] != 0, gate[0], x.reshape(-1, 8, T)).reshape(x.shape)

    def _mix(*lists):
        gate[:] = [None, None]
        _mix0(*lists)
        gate[:] = [None, None]

    def put_o(g, h, cols, val):
        if isinstance(g, int) and g == G - 1:
            _st(ot7, None, h * DH, cols, val)
        else:
            _st(ot, None, g * T + h * DH, cols, val)

    def proj(w, g, row0, nblk, buf):
        def unit(k, c):
            cols = slice(c * NC, (c + 1) * NC)
            wk = _ld(w, g, row0 + k * T, T)
            y = _dot(wk, _ld(xn, None, 0, D, cols))
            buf[k * T:(k + 1) * T, cols] = y
            mark(y)
        return [functools.partial(unit, k, c)
                for c in range(S // NC) for k in range(nblk)]

    def a_attn(g, buf, tail=False):
        def shift(h):
            for sec in (1, 2):
                rows = slice(sec * T + h * DH, sec * T + (h + 1) * DH)
                for t in range(DIL, R):
                    buf[rows, (R + t) * T:(R + t + 1) * T] = pltpu.roll(
                        buf[rows, t * T:(t + 1) * T], 1, 1)

        def unit(h, r):
            def win(sec, w):
                t = (r - DIL * w) % (2 * R)
                return buf[sec * T + h * DH:sec * T + (h + 1) * DH,
                           t * T:(t + 1) * T]
            q = win(0, 0)
            lg = compact([_fold4(q * win(1, w), jnp.add) for w in range(W)])
            lg = lg * (DH ** -0.5)
            if r < DIL * (W - 1):
                lg = jnp.where((lane == 0) & (sub * DIL > r), -1e9, lg)
            e = jnp.exp(lg - _sub_allreduce(lg, jnp.maximum))
            p = e * _recip(_sub_allreduce(e, jnp.add))
            o = None
            for w in range(W):
                term = (win(2, w).reshape(DH // 8, 8, T)
                        * jnp.broadcast_to(p[w:w + 1], (8, T)))
                o = term if o is None else o + term
            put_o(g, h, slice(r * T, (r + 1) * T), o.reshape(DH, T))
        out = []
        if tail:
            return ([functools.partial(shift, h) for h in range(T // DH)]
                    + [functools.partial(unit, h, r)
                       for r in range(R) for h in range(T // DH)])
        for h in range(T // DH):
            out.append(functools.partial(shift, h))
            out += [functools.partial(unit, h, r) for r in reversed(range(R))]
        return out

    def pipeline(mm, ew, extra=lambda g: [], top=None):
        def body(i, _):
            if top:
                pl.when(i == 1)(top)
            _mix(mm(2 * i + 1, 1), ew(2 * i, 0), extra(2 * i + 1))
            _mix(mm(2 * i + 2, 0), ew(2 * i + 1, 1), extra(2 * i + 2))
        lax.fori_loop(0, G // 2 - 1, body, None)
        _mix(mm(G - 1, 1), ew(G - 2, 0), extra(G - 1))

    def wo_unit(wo, k, c, put, lo=0, hi=D):
        cols = slice(c * NC, (c + 1) * NC)
        y = None
        if lo == 0:
            y = _dot(_ld(wo, None, k * T, T, slice(0, D - T)),
                     _ld(ot, None, 0, D - T, cols))
        if hi == D:
            y7 = _dot(_ld(wo, None, k * T, T, slice(D - T, D)),
                      _ld(ot7, None, 0, T, cols))
            y = y7 if y is None else y + y7
        put(k, c, y)
        mark(y)

    def ln(c, add=True):
        def tile(r):
            cols = slice(r * T, (r + 1) * T)
            st = {}
            blk = lambda k: xt[k * T:(k + 1) * T, cols].reshape(T // 8, 8, T)

            def mean(k):
                x = xt[k * T:(k + 1) * T, cols]
                if add:
                    x = x + ys[c % 2][k * T:(k + 1) * T, (r % n) * T:(r % n + 1) * T]
                    if c == 0:
                        x = x + yf[k // 4][:, (k % 4 * n + r) * T:(k % 4 * n + r + 1) * T]
                    xt[k * T:(k + 1) * T, cols] = x
                m = jnp.sum(pace(x).reshape(T // 8, 8, T), axis=0)
                st["m"] = m + st["m"] if k else m
                if k == G - 1:
                    st["m"] = _sub_allreduce(st["m"], jnp.add) * (1.0 / D)

            def var(k):
                d = blk(k) - pace(st["m"])
                v = jnp.sum(d * d, axis=0)
                st["v"] = v + st["v"] if k else v
                if k == G - 1:
                    v = _sub_allreduce(st["v"], jnp.add) * (1.0 / D)
                    st["v"] = lax.rsqrt(v + 1e-5)

            def norm(k):
                y = (blk(k) - pace(st["m"])) * st["v"]
                _st(xn, None, k * T, cols, y.reshape(T, T))
            return [functools.partial(f, k)
                    for f in (mean, var, norm) for k in range(G)]
        n = NC // T
        return [f for r in range(c * n, c * n + n) for f in tile(r)]

    def out_proj(wo, tail, nxt, extra=()):
        def put(k, c, y):
            ys[c % 2][k * T:(k + 1) * T, :] = y
        def add(k, c, y):
            yf[k // 4][:, (k % 4) * NC:(k % 4 + 1) * NC] = y
        mm = lambda c, f=put, lo=0, hi=D: [
            functools.partial(wo_unit, wo, k, c, f, lo, hi) for k in range(G)]
        _mix(mm(0, put, 0, D - T), tail)
        _mix(mm(0, add, D - T, D))
        for c in range(1, S // NC):
            _mix(mm(c), ln(c - 1), extra[c - 1::3])
        _mix(nxt[:len(nxt) // 2], ln(S // NC - 1))
        _mix(nxt[len(nxt) // 2:])

    a_mm = lambda g, s: proj(wa, g, 0, 3, bufs[s])
    a_ew = lambda g, s: a_attn(g, bufs[s])
    bk_mm = lambda g, s: proj(wb, g, T, 2, bufs[s])
    bq_mm = lambda g, s: proj(wb, g, 0, 1, bufs[s])

    def feature_map(paced, src, dst, c):
        def unit(h, r):
            cols = slice(r * T, (r + 1) * T)
            p = src[h * DH:(h + 1) * DH, cols] * LOG2E
            if paced:
                p = pace(p)
            for sgn, op in ((0, jnp.maximum), (1, jnp.minimum)):
                m = _sub_allreduce(_fold4(p, op), op)
                p3 = p.reshape(DH // 8, 8, T)
                e = jnp.exp2(m - p3 if sgn else p3 - m)
                inv = _recip(_sub_allreduce(jnp.sum(e, axis=0), jnp.add))
                _st(dst, None, (2 * h + sgn) * DH, cols, (e * inv).reshape(DH, T))
        n = NC // T
        return [functools.partial(unit, h, r)
                for r in range(c * n, c * n + n) for h in range(T // DH)]

    P, PR = 2 * DH, 2 * DH + 16
    rowh = lax.broadcasted_iota(jnp.int32, (PR, T), 0)
    colh = lax.broadcasted_iota(jnp.int32, (PR, T), 1) // (2 * DH)
    pair_diag = jnp.where(rowh < P, rowh // DH, rowh - P) == colh
    phi_diag = (lax.broadcasted_iota(jnp.int32, (T, T), 0) // DH
                == lax.broadcasted_iota(jnp.int32, (T, T), 1) // DH)

    def skew(fm, mm):
        out = []
        for c in range(S // NC):
            f = fm(c)
            out += f[:2]
            if c:
                out.append(functools.partial(mm, c - 1))
            out += f[2:]
        return out + [functools.partial(mm, S // NC - 1)]

    def bk_ew(g, s):
        buf, ph = bufs[s], phb[s]

        def mm(c):
            cols = slice(c * NC, (c + 1) * NC)
            for p in range(2):
                v = jnp.concatenate(
                    [buf[T + p * P:T + (p + 1) * P, cols].astype(BF16),
                     jnp.ones((PR - P, NC), BF16)], axis=0)
                kv = lax.dot_general(v, _ld(ph, None, p * T, T, cols), NT,
                                     preferred_element_type=F32)
                if c:
                    kv = kv + kvacc[p]
                if c < S // NC - 1:
                    kvacc[p] = kv
                else:
                    _st(kvt, g, p * PR, slice(None), jnp.where(pair_diag, kv, 0.0))
        return skew(functools.partial(feature_map, not isinstance(g, int) or g < G - 1, buf, ph), mm)

    def bq_ew(g, s):
        buf, ph = bufs[s], phb[s]

        def mm(c):
            cols = slice(c * NC, (c + 1) * NC)
            for p in range(2):
                nd = _dot(_ld(kvt, g, p * PR, PR), _ld(ph, None, p * T, T, cols))
                inv = 1.0 / (nd[P:P + 8] + 1e-6)
                for j in range(2):
                    put_o(g, 2 * p + j, cols,
                          nd[j * DH:(j + 1) * DH] * inv[j:j + 1])
        return skew(functools.partial(feature_map, False, buf, ph), mm)

    def store(j, src):
        def unit(m):
            def bits(r):
                t = xt[_rows(2 * j * T, 2 * T), r * T:(r + 1) * T]
                t = t + src[:, r * T:(r + 1) * T]
                return pltpu.bitcast(t.astype(BF16).astype(F32), jnp.uint32)
            xio32[j, pl.ds(m, T, stride=R // 2), :] = (
                (bits(2 * m) >> 16) | bits(2 * m + 1)).T
        return [functools.partial(unit, m) for m in range(R // 2)]

    def ocopy(j):
        c0 = j * T if isinstance(j, int) else pl.multiple_of(j * T, T)
        return pltpu.make_async_copy(xio.at[j], out_hbm.at[:, pl.ds(c0, T)],
                                     sems.at[5])

    def final_proj(tail):
        def mm(k, s, lo=0, hi=D):
            def put(k, c, y):
                if lo:
                    y = y + yf[s][:, c * NC:(c + 1) * NC]
                yf[s][:, c * NC:(c + 1) * NC] = y
            return [functools.partial(wo_unit, wbo, k, c, put, lo, hi)
                    for c in range(S // NC)]
        _mix(mm(0, 0, 0, D - T), tail)
        _mix(mm(0, 0, D - T, D))
        _mix(mm(1, 1), store(0, yf[0]))

        def body(i, _):
            ocopy(2 * i - 2).start()
            _mix(mm(2 * i, 0), store(2 * i - 1, yf[1]))
            _mix(mm(2 * i + 1, 1), store(2 * i, yf[0]))

            @pl.when(pl.program_id(0) == 0)
            def _():
                ocopy(2 * i - 1).start()
        lax.fori_loop(1, G // 2, body, None)
        ocopy(G - 2).start()
        _mix(store(G - 1, yf[1]))
        pl.when(pl.program_id(0) == 0)(ocopy(G - 1).start)
        wait([ocopy(k) for k in range(G)])

    def layer_b(last):
        with jax.named_scope("b_kv"):
            pipeline(bk_mm, bk_ew, (lambda g: []) if last else
                     (lambda g: preps((4, g - 1), *(
                         [] if isinstance(g, int) else [(5, g + 1), (6, g + 1)]))))
            _mix(bq_mm(0, 0), bk_ew(G - 1, 1), [] if last else preps((4, G - 1)))
        with jax.named_scope("b_q"):
            pipeline(bq_mm, bq_ew, (lambda g: []) if last else
                     (lambda g: preps((7, g - 1), *([(7, g)] * isinstance(g, int)))))
        with jax.named_scope("b_out"):
            if last:
                final_proj(bq_ew(G - 1, 1))
            else:
                out_proj(wbo, bq_ew(G - 1, 1), a_mm(0, 0))

    with jax.named_scope("load_x"):
        issue = [[cp] for cp in xcopy] + [[], [], second]
        start(first + issue[0] + issue[1] + issue[2])
        for j in range(G):
            wait(issue[j])
            start(issue[j + 3])
            load_x(j)
            if j == 0:
                wait(first)
                _mix(preps((0, 0), (1, 0), (2, 0)))
        _mix(ln(0, False))
        for c in range(4):
            if c == 2:
                wait(second)
                start(rest_a)
            _mix(a_mm(0, 0)[3 * c:3 * c + 3],
                 ln(c + 1, False) if c < 3 else preps((0, 1), (1, 1), (2, 1)))

    def a_prep(g):
        return preps(*([(k, g + 1) for k in range(3)] if not isinstance(g, int) else [(3, g)]),
                     (3, g - 1))

    for last in (False, True):
        with jax.named_scope("a_attn"):
            if last:
                pipeline(a_mm, a_ew)
            else:
                pipeline(a_mm, a_ew, a_prep,
                         lambda: (wait(rest_a), start(all_b)) and None)
            if not last:
                wait(all_b)
        with jax.named_scope("a_out"):
                out_proj(wao, a_attn(G - 1, bufs[1], True), bk_mm(0, 0),
                     () if last else preps((5, 0), (6, 0), (5, 1), (6, 1)))
        layer_b(last)


@jax.jit
def pallas_interleave_layers__sliding_local_dilated__linear_kernel_hedgehog__prompt_kernel(
    A_x, A_wqkv, A_wo, B_x, B_wqkv, B_w_phi, B_wo):
    del B_x
    vmem = pltpu.VMEM
    out = pl.pallas_call(
        _kernel,
        grid=(1,),
        out_shape=jax.ShapeDtypeStruct((S, D), BF16),
        in_specs=[pl.BlockSpec(memory_space=pl.ANY)] * 7,
        out_specs=pl.BlockSpec(memory_space=pl.ANY),
        scratch_shapes=[
            vmem((G, S, T), BF16),
            vmem((8, D, D), BF16),
            vmem((D, DH), BF16),
            vmem((D, S), F32),
            vmem((D // 2, S), jnp.uint32),
            vmem(((D - T) // 2, S), jnp.uint32),
            vmem((T // 2, S), jnp.uint32),
            vmem((G, 3 * T // 2, D), jnp.uint32),
            vmem((D // 2, D), jnp.uint32),
            vmem((G, 3 * T // 2, D), jnp.uint32),
            vmem((D // 2, D), jnp.uint32),
            vmem((3 * T, 2 * S), F32),
            vmem((3 * T, 2 * S), F32),
            vmem((T, S), jnp.uint32),
            vmem((T, S), jnp.uint32),
            vmem((G, 2 * DH + 16, T), jnp.uint32),
            vmem((2, 2 * DH + 16, T), F32),
            vmem((D, NC), F32), vmem((D, NC), F32),
            vmem((T, S), F32), vmem((T, S), F32),
            vmem((8, T), jnp.int32),
            pltpu.SemaphoreType.DMA((7 + G,)),
        ],
        compiler_params=pltpu.CompilerParams(
            vmem_limit_bytes=112 * 1024 * 1024),
    )(A_x.reshape(S, D), A_wqkv, A_wo, B_wqkv, B_w_phi.reshape(D, DH), B_wo,
      np.zeros((8, T), np.int32))
    return out.reshape(1, S, D)
```

```python
import functools

import jax
import numpy as np
import jax.numpy as jnp
from jax import lax
import jax.experimental.pallas as pl
import jax.experimental.pallas.tpu as pltpu

S, D, H, DH, W, DIL = 2048, 1024, 32, 32, 8, 2
T = 128
R = S // T
G = D // T
NC = 512
F32, BF16 = jnp.float32, jnp.bfloat16
LOG2E = 1.4426950408889634
NT = (((1,), (1,)), ((), ()))


def _dot(a, b):
    return jnp.dot(a, b, preferred_element_type=F32)


def _rows(row, n):
    if isinstance(row, int):
        return pl.ds(row // 2, n // 2)
    return pl.ds(pl.multiple_of(row // 2, 8), n // 2)


def _ld(ref, g, row, n, cols=slice(None)):
    idx = (_rows(row, n), cols) if g is None else (g, _rows(row, n), cols)
    return pltpu.bitcast(ref[idx], BF16)


def _st(ref, g, row, cols, val):
    rows = _rows(row, val.shape[0])
    idx = (rows, cols) if g is None else (g, rows, cols)
    ref[idx] = pltpu.bitcast(val.astype(BF16), jnp.uint32)


def _mix0(*lists):
    items = [((i + 0.5) / len(l), j, f)
             for j, l in enumerate(lists) for i, f in enumerate(l)]
    for _, _, f in sorted(items, key=lambda t: t[:2]):
        f()


def _sub_allreduce(x, op):
    for d in (4, 2, 1):
        x = op(x, pltpu.roll(x, d, 0))
    return x


def _recip(s):
    r = pl.reciprocal(s, approx=True)
    return r * (2.0 - s * r)


def _fold4(x, op):
    return op(op(x[0:8], x[8:16]), op(x[16:24], x[24:32]))


def _kernel(x_hbm, awqkv_hbm, awo_hbm, bwqkv_hbm, phi_hbm, bwo_hbm, zeros_hbm,
            out_hbm,
            xio, stage, phis, xt, xn, ot, ot7, wa, wao, wb, wbo, buf0, buf1,
            ph0, ph1, kvt, kvacc, y0, y1, yf0, yf1, zeros_ref, sems):

    def wcopy(k, lo, n, sem):
        src = (awqkv_hbm, awqkv_hbm, awqkv_hbm, awo_hbm,
               bwqkv_hbm, bwqkv_hbm, bwqkv_hbm, bwo_hbm)[k]
        src = src.at[:, pl.ds((k % 4) * D * (k % 4 != 3) + lo, n)]
        return pltpu.make_async_copy(src, stage.at[k, :, pl.ds(lo, n)],
                                     sems.at[sem])

    xcopy = [pltpu.make_async_copy(x_hbm.at[:, pl.ds(j * T, T)], xio.at[j],
                                   sems.at[7 + j]) for j in range(G)]
    first = [wcopy(k, 0, T, 1) for k in range(3)]
    second = [wcopy(k, T, T, 2) for k in range(3)]
    first.append(pltpu.make_async_copy(zeros_hbm, zeros_ref, sems.at[1]))
    second += [wcopy(k, 2 * T, 2 * T, 2) for k in range(3)]
    second.append(wcopy(3, 0, 2 * T, 2))
    rest_a = [wcopy(k, 4 * T, D - 4 * T, 3) for k in range(3)]
    rest_a.append(wcopy(3, 2 * T, D - 2 * T, 3))
    all_b = [wcopy(k, 0, D, 4) for k in range(4, 8)]
    all_b.append(pltpu.make_async_copy(phi_hbm, phis, sems.at[4]))

    def start(cps):
        for cp in cps:
            cp.start()

    def wait(cps):
        for cp in cps:
            cp.wait()

    xio32 = xio.bitcast(jnp.uint32)
    hi_mask = jnp.uint32(0xFFFF0000)

    def load_x(j):
        for m in range(R // 2):
            u = xio32[j, pl.ds(m, T, stride=R // 2), :].T
            for par, bits in enumerate((u << 16, u & hi_mask)):
                r = 2 * m + par
                xt[j * T:(j + 1) * T, r * T:(r + 1) * T] = pltpu.bitcast(bits, F32)

    def wt(k, g):
        c0 = g * T if isinstance(g, int) else pl.multiple_of(g * T, T)
        return stage[k, :, pl.ds(c0, T)].T

    def prep(k, g):
        dst, gi, row = (((wa, g, k * T),) * 3 + ((wao, None, g * T),)
                        + ((wb, g, k * T - 4 * T),) * 3 + ((wbo, None, g * T),))[k]
        w = wt(k, g)
        if k in (4, 5):
            r0 = g * T if isinstance(g, int) else pl.multiple_of(g * T, T)
            rows = phis[pl.ds(r0, T), :]
            bd = jnp.where(phi_diag, jnp.concatenate([rows] * 4, axis=1), 0)
            w = _dot(bd.astype(F32).T.astype(BF16), w)
        _st(dst, gi, row, slice(None), w)

    def preps(*kg):
        return [functools.partial(prep, k, g) for k, g in kg]

    sub = lax.broadcasted_iota(jnp.int32, (8, T), 0)
    lane = lax.broadcasted_iota(jnp.int32, (8, T), 1)
    bufs = (buf0, buf1)
    ys, yf = (y0, y1), (yf0, yf1)
    phb = (ph0, ph1)

    def compact(ps):
        for d in (4, 2, 1):
            clear = (sub & d) == 0
            nxt = []
            for j in range(d):
                a, b = ps[j], ps[j + d]
                if d == 4:
                    nxt.append(jnp.where(clear, a, b)
                               + pltpu.roll(jnp.where(clear, b, a), 4, 0))
                else:
                    nxt.append(jnp.where(clear, a + pltpu.roll(a, 8 - d, 0),
                                         b + pltpu.roll(b, d, 0)))
            ps = nxt
        return ps[0]

    gate = [None, None]

    def mark(y):
        gate[:] = [gate[1], y[-8:, -T:]]

    def pace(x):
        if gate[0] is None:
            return x
        return jnp.where(zeros_ref[...] != 0, gate[0], x.reshape(-1, 8, T)).reshape(x.shape)

    def _mix(*lists):
        gate[:] = [None, None]
        _mix0(*lists)
        gate[:] = [None, None]

    def put_o(g, h, cols, val):
        if isinstance(g, int) and g == G - 1:
            _st(ot7, None, h * DH, cols, val)
        else:
            _st(ot, None, g * T + h * DH, cols, val)

    def proj(w, g, row0, nblk, buf):
        def unit(k, c):
            cols = slice(c * NC, (c + 1) * NC)
            wk = _ld(w, g, row0 + k * T, T)
            y = _dot(wk, _ld(xn, None, 0, D, cols))
            buf[k * T:(k + 1) * T, cols] = y
            mark(y)
        return [functools.partial(unit, k, c)
                for c in range(S // NC) for k in range(nblk)]

    def a_attn(g, buf, tail=False):
        def shift(h):
            for sec in (1, 2):
                rows = slice(sec * T + h * DH, sec * T + (h + 1) * DH)
                for t in range(DIL, R):
                    buf[rows, (R + t) * T:(R + t + 1) * T] = pltpu.roll(
                        buf[rows, t * T:(t + 1) * T], 1, 1)

        def unit(h, r):
            def win(sec, w):
                t = (r - DIL * w) % (2 * R)
                return buf[sec * T + h * DH:sec * T + (h + 1) * DH,
                           t * T:(t + 1) * T]
            q = win(0, 0)
            lg = compact([_fold4(q * win(1, w), jnp.add) for w in range(W)])
            lg = lg * (DH ** -0.5)
            if r < DIL * (W - 1):
                lg = jnp.where((lane == 0) & (sub * DIL > r), -1e9, lg)
            e = jnp.exp(lg - _sub_allreduce(lg, jnp.maximum))
            p = e * _recip(_sub_allreduce(e, jnp.add))
            o = None
            for w in range(W):
                term = (win(2, w).reshape(DH // 8, 8, T)
                        * jnp.broadcast_to(p[w:w + 1], (8, T)))
                o = term if o is None else o + term
            put_o(g, h, slice(r * T, (r + 1) * T), o.reshape(DH, T))
        out = [functools.partial(shift, h) for h in range(T // DH)]
        if tail:
            return out + [functools.partial(unit, h, r)
                          for r in range(R) for h in range(T // DH)]
        for h in range(T // DH):
            out += [functools.partial(unit, h, r) for r in reversed(range(R))]
        return out

    def pipeline(mm, ew, extra=lambda g: [], top=None):
        def body(i, _):
            if top:
                pl.when(i == 1)(top)
            _mix(mm(2 * i + 1, 1), ew(2 * i, 0), extra(2 * i + 1))
            _mix(mm(2 * i + 2, 0), ew(2 * i + 1, 1), extra(2 * i + 2))
        lax.fori_loop(0, G // 2 - 1, body, None)
        _mix(mm(G - 1, 1), ew(G - 2, 0), extra(G - 1))

    def wo_unit(wo, k, c, put, lo=0, hi=D):
        cols = slice(c * NC, (c + 1) * NC)
        y = None
        if lo == 0:
            y = _dot(_ld(wo, None, k * T, T, slice(0, D - T)),
                     _ld(ot, None, 0, D - T, cols))
        if hi == D:
            y7 = _dot(_ld(wo, None, k * T, T, slice(D - T, D)),
                      _ld(ot7, None, 0, T, cols))
            y = y7 if y is None else y + y7
        put(k, c, y)
        mark(y)

    def ln(c, add=True):
        def tile(r):
            cols = slice(r * T, (r + 1) * T)
            st = {}
            blk = lambda k: xt[k * T:(k + 1) * T, cols].reshape(T // 8, 8, T)

            def mean(k):
                x = xt[k * T:(k + 1) * T, cols]
                if add:
                    x = x + ys[c % 2][k * T:(k + 1) * T, (r % n) * T:(r % n + 1) * T]
                    if c == 0:
                        x = x + yf[k // 4][:, (k % 4 * n + r) * T:(k % 4 * n + r + 1) * T]
                    xt[k * T:(k + 1) * T, cols] = x
                m = jnp.sum(pace(x).reshape(T // 8, 8, T), axis=0)
                st["m"] = m + st["m"] if k else m
                if k == G - 1:
                    st["m"] = _sub_allreduce(st["m"], jnp.add) * (1.0 / D)

            def var(k):
                d = blk(k) - pace(st["m"])
                v = jnp.sum(d * d, axis=0)
                st["v"] = v + st["v"] if k else v
                if k == G - 1:
                    v = _sub_allreduce(st["v"], jnp.add) * (1.0 / D)
                    st["v"] = lax.rsqrt(v + 1e-5)

            def norm(k):
                y = (blk(k) - pace(st["m"])) * st["v"]
                _st(xn, None, k * T, cols, y.reshape(T, T))
            return [functools.partial(f, k)
                    for f in (mean, var, norm) for k in range(G)]
        n = NC // T
        return [f for r in range(c * n, c * n + n) for f in tile(r)]

    def out_proj(wo, tail, nxt, extra=()):
        def put(k, c, y):
            ys[c % 2][k * T:(k + 1) * T, :] = y
        def add(k, c, y):
            yf[k // 4][:, (k % 4) * NC:(k % 4 + 1) * NC] = y
        mm = lambda c, f=put, lo=0, hi=D: [
            functools.partial(wo_unit, wo, k, c, f, lo, hi) for k in range(G)]
        _mix(mm(0, put, 0, D - T), tail)
        _mix(mm(0, add, D - T, D))
        for c in range(1, S // NC):
            _mix(mm(c), ln(c - 1), extra[c - 1::3])
        _mix(nxt[:len(nxt) // 2], ln(S // NC - 1))
        _mix(nxt[len(nxt) // 2:])

    a_mm = lambda g, s: proj(wa, g, 0, 3, bufs[s])
    a_ew = lambda g, s: a_attn(g, bufs[s])
    bk_mm = lambda g, s: proj(wb, g, T, 2, bufs[s])
    bq_mm = lambda g, s: proj(wb, g, 0, 1, bufs[s])

    def feature_map(paced, src, dst, c):
        def unit(h, r):
            cols = slice(r * T, (r + 1) * T)
            p = src[h * DH:(h + 1) * DH, cols] * LOG2E
            if paced:
                p = pace(p)
            for sgn, op in ((0, jnp.maximum), (1, jnp.minimum)):
                m = _sub_allreduce(_fold4(p, op), op)
                p3 = p.reshape(DH // 8, 8, T)
                e = jnp.exp2(m - p3 if sgn else p3 - m)
                inv = _recip(_sub_allreduce(jnp.sum(e, axis=0), jnp.add))
                _st(dst, None, (2 * h + sgn) * DH, cols, (e * inv).reshape(DH, T))
        n = NC // T
        return [functools.partial(unit, h, r)
                for r in range(c * n, c * n + n) for h in range(T // DH)]

    P, PR = 2 * DH, 2 * DH + 16
    rowh = lax.broadcasted_iota(jnp.int32, (PR, T), 0)
    colh = lax.broadcasted_iota(jnp.int32, (PR, T), 1) // (2 * DH)
    pair_diag = jnp.where(rowh < P, rowh // DH, rowh - P) == colh
    phi_diag = (lax.broadcasted_iota(jnp.int32, (T, T), 0) // DH
                == lax.broadcasted_iota(jnp.int32, (T, T), 1) // DH)

    def skew(fm, mm):
        out = []
        for c in range(S // NC):
            f = fm(c)
            out += f[:2]
            if c:
                out.append(functools.partial(mm, c - 1))
            out += f[2:]
        return out + [functools.partial(mm, S // NC - 1)]

    def bk_ew(g, s):
        buf, ph = bufs[s], phb[s]

        def mm(c):
            cols = slice(c * NC, (c + 1) * NC)
            for p in range(2):
                v = jnp.concatenate(
                    [buf[T + p * P:T + (p + 1) * P, cols].astype(BF16),
                     jnp.ones((PR - P, NC), BF16)], axis=0)
                kv = lax.dot_general(v, _ld(ph, None, p * T, T, cols), NT,
                                     preferred_element_type=F32)
                if c:
                    kv = kv + kvacc[p]
                if c < S // NC - 1:
                    kvacc[p] = kv
                else:
                    _st(kvt, g, p * PR, slice(None), jnp.where(pair_diag, kv, 0.0))
        return skew(functools.partial(feature_map, not isinstance(g, int) or g < G - 1, buf, ph), mm)

    def bq_ew(g, s):
        buf, ph = bufs[s], phb[s]

        def mm(c):
            cols = slice(c * NC, (c + 1) * NC)
            for p in range(2):
                nd = _dot(_ld(kvt, g, p * PR, PR), _ld(ph, None, p * T, T, cols))
                inv = 1.0 / (nd[P:P + 8] + 1e-6)
                for j in range(2):
                    put_o(g, 2 * p + j, cols,
                          nd[j * DH:(j + 1) * DH] * inv[j:j + 1])
        return skew(functools.partial(feature_map, False, buf, ph), mm)

    def store(j, src):
        def unit(m):
            def bits(r):
                t = xt[_rows(2 * j * T, 2 * T), r * T:(r + 1) * T]
                t = t + src[:, r * T:(r + 1) * T]
                return pltpu.bitcast(t.astype(BF16).astype(F32), jnp.uint32)
            xio32[j, pl.ds(m, T, stride=R // 2), :] = (
                (bits(2 * m) >> 16) | bits(2 * m + 1)).T
        return [functools.partial(unit, m) for m in range(R // 2)]

    def ocopy(j):
        c0 = j * T if isinstance(j, int) else pl.multiple_of(j * T, T)
        return pltpu.make_async_copy(xio.at[j], out_hbm.at[:, pl.ds(c0, T)],
                                     sems.at[5])

    def final_proj(tail):
        def mm(k, s, lo=0, hi=D):
            def put(k, c, y):
                if lo:
                    y = y + yf[s][:, c * NC:(c + 1) * NC]
                yf[s][:, c * NC:(c + 1) * NC] = y
            return [functools.partial(wo_unit, wbo, k, c, put, lo, hi)
                    for c in range(S // NC)]
        _mix(mm(0, 0, 0, D - T), tail)
        _mix(mm(0, 0, D - T, D))
        _mix(mm(1, 1), store(0, yf[0]))

        def body(i, _):
            ocopy(2 * i - 2).start()
            _mix(mm(2 * i, 0), store(2 * i - 1, yf[1]))
            _mix(mm(2 * i + 1, 1), store(2 * i, yf[0]))

            @pl.when(pl.program_id(0) == 0)
            def _():
                ocopy(2 * i - 1).start()
        lax.fori_loop(1, G // 2, body, None)
        ocopy(G - 2).start()
        _mix(store(G - 1, yf[1]))
        pl.when(pl.program_id(0) == 0)(ocopy(G - 1).start)
        wait([ocopy(k) for k in range(G)])

    def layer_b(last):
        with jax.named_scope("b_kv"):
            pipeline(bk_mm, bk_ew, (lambda g: []) if last else
                     (lambda g: preps((4, g - 1), *(
                         [] if isinstance(g, int) else [(5, g + 1), (6, g + 1)]))))
            _mix(bq_mm(0, 0), bk_ew(G - 1, 1), [] if last else preps((4, G - 1)))
        with jax.named_scope("b_q"):
            pipeline(bq_mm, bq_ew, (lambda g: []) if last else
                     (lambda g: preps((7, g - 1), *([(7, g)] * isinstance(g, int)))))
        with jax.named_scope("b_out"):
            if last:
                final_proj(bq_ew(G - 1, 1))
            else:
                out_proj(wbo, bq_ew(G - 1, 1), a_mm(0, 0))

    with jax.named_scope("load_x"):
        issue = [[cp] for cp in xcopy] + [[], [], second]
        start(first + issue[0] + issue[1] + issue[2])
        for j in range(G):
            wait(issue[j])
            start(issue[j + 3])
            load_x(j)
            if j == 0:
                wait(first)
                _mix(preps((0, 0), (1, 0), (2, 0)))
        _mix(ln(0, False))
        for c in range(4):
            if c == 2:
                wait(second)
                start(rest_a)
            _mix(a_mm(0, 0)[3 * c:3 * c + 3],
                 ln(c + 1, False) if c < 3 else preps((0, 1), (1, 1), (2, 1)))

    def a_prep(g):
        return preps(*([(k, g + 1) for k in range(3)] if not isinstance(g, int) else [(3, g)]),
                     (3, g - 1))

    for last in (False, True):
        with jax.named_scope("a_attn"):
            if last:
                pipeline(a_mm, a_ew)
            else:
                pipeline(a_mm, a_ew, a_prep,
                         lambda: (wait(rest_a), start(all_b)) and None)
            if not last:
                wait(all_b)
        with jax.named_scope("a_out"):
                out_proj(wao, a_attn(G - 1, bufs[1], True), bk_mm(0, 0),
                     () if last else preps((5, 0), (6, 0), (5, 1), (6, 1)))
        layer_b(last)


@jax.jit
def pallas_interleave_layers__sliding_local_dilated__linear_kernel_hedgehog__prompt_kernel(
    A_x, A_wqkv, A_wo, B_x, B_wqkv, B_w_phi, B_wo):
    del B_x
    vmem = pltpu.VMEM
    out = pl.pallas_call(
        _kernel,
        grid=(1,),
        out_shape=jax.ShapeDtypeStruct((S, D), BF16),
        in_specs=[pl.BlockSpec(memory_space=pl.ANY)] * 7,
        out_specs=pl.BlockSpec(memory_space=pl.ANY),
        scratch_shapes=[
            vmem((G, S, T), BF16),
            vmem((8, D, D), BF16),
            vmem((D, DH), BF16),
            vmem((D, S), F32),
            vmem((D // 2, S), jnp.uint32),
            vmem(((D - T) // 2, S), jnp.uint32),
            vmem((T // 2, S), jnp.uint32),
            vmem((G, 3 * T // 2, D), jnp.uint32),
            vmem((D // 2, D), jnp.uint32),
            vmem((G, 3 * T // 2, D), jnp.uint32),
            vmem((D // 2, D), jnp.uint32),
            vmem((3 * T, 2 * S), F32),
            vmem((3 * T, 2 * S), F32),
            vmem((T, S), jnp.uint32),
            vmem((T, S), jnp.uint32),
            vmem((G, 2 * DH + 16, T), jnp.uint32),
            vmem((2, 2 * DH + 16, T), F32),
            vmem((D, NC), F32), vmem((D, NC), F32),
            vmem((T, S), F32), vmem((T, S), F32),
            vmem((8, T), jnp.int32),
            pltpu.SemaphoreType.DMA((7 + G,)),
        ],
        compiler_params=pltpu.CompilerParams(flags={"XLA_TPU_EVENLY_DISTRIBUTE_CRITICAL_NODES": True},
            vmem_limit_bytes=112 * 1024 * 1024),
    )(A_x.reshape(S, D), A_wqkv, A_wo, B_wqkv, B_w_phi.reshape(D, DH), B_wo,
      np.zeros((8, T), np.int32))
    return out.reshape(1, S, D)
```
